```python
import jax
import jax.numpy as jnp

def _softmax(x, axis=-1):
    return jax.nn.softmax(x, axis=axis)
def _gelu(x):
    return jax.nn.gelu(x, approximate=True)
def _silu(x):
    return jax.nn.silu(x)
def _sigmoid(x):
    return jax.nn.sigmoid(x)
def _layernorm(x, axis=-1, eps=1e-5):
    m = jnp.mean(x, axis=axis, keepdims=True)
    v = jnp.var(x, axis=axis, keepdims=True)
    return (x - m) / jnp.sqrt(v + eps)
def _scatter_add(tgt, idx, src, axis=0):
    return tgt.at[idx].add(src)
def _segment_sum(src, seg, n):
    return jax.ops.segment_sum(src, seg, n)
class _Rng:
    def __init__(self, key):
        self._k = key
    def _next(self):
        self._k, sub = jax.random.split(self._k)
        return sub
    def normal(self, shape):
        return jax.random.normal(self._next(), shape, dtype=jnp.bfloat16)
    def randint(self, lo, hi, shape):
        return jax.random.randint(self._next(), shape, lo, hi, dtype=jnp.int32)
    def uniform(self, shape, lo=0.0, hi=1.0):
        return jax.random.uniform(self._next(), shape, jnp.bfloat16, lo, hi)
    def permutation(self, n):
        return jax.random.permutation(self._next(), n)


kernel_name = 'interleave_layers__ssm_conv_h3__mixer_s_mlp__prompt'

def setup_inputs():
    _rng = _Rng(jax.random.key(int.from_bytes(__import__("os").urandom(4), "little")))
    _w = (lambda a: (lambda t: t.astype(jnp.bfloat16) if jnp.issubdtype(t.dtype, jnp.floating) else t)(jnp.asarray(a)))
    def _A_setup():
        B, S, D = 1, 2048, 1024
        ks = 4
        return {
            "q": _w((lambda *s: _rng.normal(s) * 0.05)(B, S, D)),
            "k": _w((lambda *s: _rng.normal(s) * 0.05)(B, S, D)),
            "v": _w((lambda *s: _rng.normal(s) * 0.05)(B, S, D)),
            "shift_k": _w((lambda *s: _rng.normal(s) * 0.05)(D, ks) * 0.5),
            "ssm_k": _w((lambda *s: _rng.normal(s) * 0.05)(D, S) * (1.0 / S ** 0.5)),
            "ssm_D": _w((lambda *s: _rng.normal(s) * 0.05)(D)),
        }
    _A_in = _A_setup()

    def _B_setup():
        B, S, D, F = 1, 2048, 1024, 3584
        return {
            "x":  _w((lambda *s: _rng.normal(s) * 0.05)(B, S, D)),
            "w1": _w((lambda *s: _rng.normal(s) * 0.05)(D, D) * (D ** -0.5)),
            "w2": _w((lambda *s: _rng.normal(s) * 0.05)(D, D) * (D ** -0.5)),
            "w3": _w((lambda *s: _rng.normal(s) * 0.05)(D, F) * (D ** -0.5)),
            "w4": _w((lambda *s: _rng.normal(s) * 0.05)(F, D) * (F ** -0.5)),
        }
    _B_in = _B_setup()

    return {
        "A_q": _A_in["q"],
        "A_k": _A_in["k"],
        "A_v": _A_in["v"],
        "A_shift_k": _A_in["shift_k"],
        "A_ssm_k": _A_in["ssm_k"],
        "A_ssm_D": _A_in["ssm_D"],
        "B_x": _B_in["x"],
        "B_w1": _B_in["w1"],
        "B_w2": _B_in["w2"],
        "B_w3": _B_in["w3"],
        "B_w4": _B_in["w4"],
    }

def reference(A_q, A_k, A_v, A_shift_k, A_ssm_k, A_ssm_D, B_x, B_w1, B_w2, B_w3, B_w4):
    def _A_ref(q, k, v, shift_k, ssm_k, ssm_D):
        B, S, D = q.shape
        ks = shift_k.shape[-1]
        k_pad = jnp.pad(k, ((0, 0), (ks - 1, 0), (0, 0)))
        k_shift = jnp.zeros_like(k)
        for t in range(ks):
            k_shift = k_shift + k_pad[:, t:t + S, :] * shift_k[:, ks - 1 - t][None, None, :]
        kv = k_shift * v
        L = 2 * S
        kv_pad = jnp.pad(kv, ((0, 0), (0, S), (0, 0)))
        kf_pad = jnp.pad(ssm_k, ((0, 0), (0, S)))
        kv_f = (lambda x, axes=(-2,-1): jnp.fft.rfft2(x.astype(jnp.float32), axes=axes))(kv_pad[:, None, :, :], axes=(1, 2))
        kf_f = (lambda x, axes=(-2,-1): jnp.fft.rfft2(x.astype(jnp.float32), axes=axes))(kf_pad[:, None, :], axes=(1, 2))
        kf_f = (lambda x, *d: x.transpose(*d))(kf_f, 1, 2, 0)
        y_f = kv_f * kf_f[None, :, :, :]
        y = (lambda x, s, axes=(-2,-1): jnp.fft.irfft2(x, s=s, axes=axes).astype(jnp.bfloat16))(y_f, (1, L), axes=(1, 2))[:, 0, :S, :]
        y = y + kv * ssm_D[None, None, :]
        return q * y

    def _B_ref(x, w1, w2, w3, w4):
        B, S, D = x.shape
        h = _gelu(_layernorm(x, axis=-1) @ w1)
        c = D // 4
        g0 = jnp.pad(h[:, :, 0*c:1*c], ((0, 0), (1, 0), (0, 0)))[:, :S, :]
        g1 = jnp.pad(h[:, :, 1*c:2*c], ((0, 0), (0, 1), (0, 0)))[:, 1:, :]
        g2 = jnp.pad(h[:, :, 2*c:3*c], ((0, 0), (2, 0), (0, 0)))[:, :S, :]
        g3 = jnp.pad(h[:, :, 3*c:   ], ((0, 0), (0, 2), (0, 0)))[:, 2:, :]
        hs = jnp.concatenate([g0, g1, g2, g3], axis=-1) @ w2
        x1 = x + hs
        h2 = _gelu(_layernorm(x1, axis=-1) @ w3) @ w4
        return x1 + h2

    x = A_q
    x = x + _A_ref(_layernorm(x, axis=-1), A_k, A_v, A_shift_k, A_ssm_k, A_ssm_D)
    x = x + _B_ref(_layernorm(x, axis=-1), B_w1, B_w2, B_w3, B_w4)
    x = x + _A_ref(_layernorm(x, axis=-1), A_k, A_v, A_shift_k, A_ssm_k, A_ssm_D)
    x = x + _B_ref(_layernorm(x, axis=-1), B_w1, B_w2, B_w3, B_w4)
    return x
```

```python
import functools
import math

import jax
import jax.numpy as jnp
from jax import lax
import jax.experimental.pallas as pl
import jax.experimental.pallas.tpu as pltpu

S = 2048
D = 1024
F = 3584
TM = 256
T = S // TM
PB = 128
NB = S // PB
C4 = D // 4
EPS = 1e-5
SHIFTS = (1, -1, 2, -2)
f32 = jnp.float32
bf16 = jnp.bfloat16


def _ln(x):
    m = jnp.mean(x, axis=-1, keepdims=True)
    xc = x - m
    v = jnp.mean(xc * xc, axis=-1, keepdims=True)
    return xc * lax.rsqrt(v + EPS)


def _gelu(x):
    c = math.sqrt(2.0 / math.pi)
    inner = x * (c + (c * 0.044715) * (x * x))
    hx = 0.5 * x
    return hx + hx * jnp.tanh(inner)


def _dot(a, b):
    return jnp.dot(a, b, preferred_element_type=f32)


def _dot_nt(a, b):
    return lax.dot_general(a, b, (((1,), (1,)), ((), ())), preferred_element_type=f32)


def _dft_angle(r, t):
    rr = r & 127
    fr = jnp.where(rr < 64, 2 * rr, 2 * rr - 127)
    m = ((2 * fr + 1) * t + jnp.where(r >= 128, 128, 0)) & 511
    return m.astype(f32) * (2.0 * math.pi / 512.0)


def _pieces(val, n_lo=0, n_hi=None, ngroup=1):
    rows, cols = val.shape
    nt = cols // 128
    n_hi = nt if n_hi is None else n_hi
    out = []
    for n0 in range(n_lo, n_hi, ngroup):
        for r in range(rows // 8):
            out.append(val[r * 8:(r + 1) * 8, n0 * 128:(n0 + 1) * 128])
    return out


def _pick(srcs, n):
    if not srcs:
        return [None] * n
    return [srcs[(i * len(srcs)) // n] for i in range(n)]


def make(FC=512, only=None, trig_b=6, mac_rows=16, mac_lanes=256, nr_hi=6, np_hi=7):
    NFC = F // FC

    def kernel(q_hbm, k_hbm, v_hbm, sk_hbm, hk_hbm, dv_hbm, w1_hbm, w2_hbm, w3_hbm, w4_hbm,
               o_hbm,
               qb, kb, vb, hkb, w1, w2, w3, w4, sk_ref, dv_ref, ff, fi, skt, kcar, hprev, U, G, Yb,
               ybuf, hs3, xab, xinb, baseb, zbuf, obuf,
               sem_in, sem_w, sem_o):
        def in_copies(j):
            rows = pl.ds(j * TM, TM)
            sl = j % 2
            return [
                pltpu.make_async_copy(hk_hbm.at[:, rows], hkb.at[sl], sem_in.at[0, j]),
                pltpu.make_async_copy(k_hbm.at[0, rows, :], kb.at[sl], sem_in.at[1, j]),
                pltpu.make_async_copy(v_hbm.at[0, rows, :], vb.at[sl], sem_in.at[2, j]),
                pltpu.make_async_copy(q_hbm.at[0, rows, :], qb.at[rows, :], sem_in.at[3, j]),
            ]

        w_copies = [
            pltpu.make_async_copy(w1_hbm, w1, sem_w.at[0]),
            pltpu.make_async_copy(w2_hbm, w2, sem_w.at[1]),
            pltpu.make_async_copy(w3_hbm, w3, sem_w.at[2]),
            pltpu.make_async_copy(w4_hbm, w4, sem_w.at[3]),
            pltpu.make_async_copy(sk_hbm, sk_ref, sem_w.at[4]),
            pltpu.make_async_copy(dv_hbm, dv_ref, sem_w.at[5]),
        ]

        def out_copy(j):
            rows = pl.ds(j * TM, TM)
            return pltpu.make_async_copy(obuf.at[rows, :], o_hbm.at[0, rows, :], sem_o.at[j])

        z = jnp.min(lax.broadcasted_iota(jnp.int32, (8, 128), 1))
        never = z > 0
        z16 = pl.multiple_of(z, 16)

        def tie(x, trig):
            if trig is None:
                return x
            head = jnp.where(never, trig, x[:8, :128])
            if x.shape[1] > 128:
                head = jnp.concatenate([head, x[:8, 128:]], axis=1)
            if x.shape[0] > 8:
                head = jnp.concatenate([head, x[8:]], axis=0)
            return head

        def prologue():
            w_copies[4].start()
            w_copies[5].start()
            for c in in_copies(0):
                c.start()
            for c in in_copies(1):
                c.start()
            w_copies[0].start()
            r = lax.broadcasted_iota(jnp.int32, (2 * PB, PB), 0)
            t = lax.broadcasted_iota(jnp.int32, (2 * PB, PB), 1)
            ff[...] = jnp.cos(_dft_angle(r, t)).astype(bf16)
            r = lax.broadcasted_iota(jnp.int32, (PB, 2 * PB), 1)
            t = lax.broadcasted_iota(jnp.int32, (PB, 2 * PB), 0)
            fi[...] = (jnp.cos(_dft_angle(r, t)) * (1.0 / PB)).astype(bf16)
            kcar[...] = jnp.zeros((8, D), f32)
            hs3[1, 0:8, :] = jnp.zeros((8, D), f32)
            hs3[T, TM - 8:TM, :] = jnp.zeros((8, D), f32)
            w_copies[4].wait()
            w_copies[5].wait()
            e = (lax.broadcasted_iota(jnp.int32, (8, 4), 0)
                 == lax.broadcasted_iota(jnp.int32, (8, 4), 1)).astype(bf16)
            skt[0:8, :] = _dot_nt(e, sk_ref[...])
            skt[8:16, :] = jnp.broadcast_to(dv_ref[...].astype(f32), (8, D))

        def conv_fwd_h(j):
            sl = j % 2
            ffv = ff[...]
            srcs = []
            hlast = None
            for i in range(2):
                b = 2 * j + i
                hh = _dot_nt(ffv, hkb[sl, :, i * PB:(i + 1) * PB])
                srcs += _pieces(hh, ngroup=4)
                gr, gi = hh[:PB], hh[PB:]
                if b > 0:
                    hp = hprev[...] if i == 0 else hlast
                    pr, pi_ = hp[:PB], hp[PB:]
                    gr = jnp.concatenate([gr[:64] - pi_[:64], gr[64:] + pi_[64:]], axis=0)
                    gi = jnp.concatenate([gi[:64] + pr[:64], gi[64:] - pr[64:]], axis=0)
                G[z + b, 0:PB, :] = gr
                G[z + b, PB:2 * PB, :] = gi - gr
                G[z + b, 2 * PB:3 * PB, :] = gr + gi
                hlast = hh
            if j < T - 1:
                hprev[...] = hlast
            return srcs

        def conv_kv(j, trigs):
            sl = j % 2
            us, kvds = [], []
            for i in range(2):
                ucols, dcols = [], []
                for lt in range(D // 128):
                    ls = slice(lt * 128, (lt + 1) * 128)
                    kf = kb[sl, i * PB:(i + 1) * PB, ls].astype(f32)
                    if i == 0:
                        prev = kcar[:, ls]
                    else:
                        prev = kb[sl, PB - 16:PB, ls].astype(f32)[8:]
                    ext = jnp.concatenate([prev, kf], axis=0)
                    s0 = tie(jnp.broadcast_to(skt[0:1, ls], (8, 128)), trigs[i * 8 + lt])
                    ks = kf * jnp.concatenate([s0] * (PB // 8), axis=0)
                    for tt in range(1, 4):
                        ks = ks + ext[8 - tt:8 - tt + PB, :] * skt[tt:tt + 1, ls]
                    kv = ks * vb[sl, i * PB:(i + 1) * PB, ls].astype(f32)
                    ucols.append(kv.astype(bf16))
                    dcols.append(kv * skt[8:9, ls])
                    if i == 1 and j < T - 1:
                        kcar[:, ls] = kf[PB - 8:]
                us.append(jnp.concatenate(ucols, axis=1))
                kvds.append(jnp.concatenate(dcols, axis=1))
            return us, kvds

        def conv_fwd_u(j, us):
            ffv = ff[...]
            srcs = []
            for i in range(2):
                uu = _dot(ffv, us[i])
                srcs += _pieces(uu, ngroup=4)
                U[z + 2 * j + i] = uu
            return srcs

        def conv_mac(j, trigs):
            a1, a2 = 2 * j, 2 * j + 1
            RG = mac_rows
            k = 0
            for r0 in range(0, PB, RG):
                for lt in range(D // mac_lanes):
                    ls = slice(lt * mac_lanes, (lt + 1) * mac_lanes)

                    def ld(ref, idx, p):
                        return ref[idx, p * PB + r0:p * PB + r0 + RG, ls]

                    gcache = {}

                    def gld(c):
                        if c not in gcache:
                            gcache[c] = [ld(G, c, p) for p in range(3)]
                        return gcache[c]

                    acc1 = acc2 = None
                    for b in range(a2 + 1):
                        ua, ub = ld(U, b, 0), ld(U, b, 1)
                        if b == 0 and trigs[k] is not None:
                            tg = jnp.concatenate([trigs[k]] * (RG // 8), axis=0)
                            tg = jnp.concatenate([tg] * (mac_lanes // 128), axis=1)
                            ua = jnp.where(never, tg, ua)
                        us = ua + ub
                        g2 = gld(a2 - b)
                        t2 = [g2[0] * us, g2[1] * ua, g2[2] * ub]
                        acc2 = t2 if acc2 is None else [x + y for x, y in zip(acc2, t2)]
                        if a1 - b >= 0:
                            g1 = gld(a1 - b)
                            t1 = [g1[0] * us, g1[1] * ua, g1[2] * ub]
                            acc1 = t1 if acc1 is None else [x + y for x, y in zip(acc1, t1)]
                    for i, acc in enumerate((acc1, acc2)):
                        Yb[i, pl.ds(z16 + r0, RG), ls] = (acc[0] - acc[2]).astype(Yb.dtype)
                        Yb[i, pl.ds(z16 + PB + r0, RG), ls] = (acc[0] + acc[1]).astype(Yb.dtype)
                    k += 1

        n_mac_tasks = (PB // mac_rows) * (D // mac_lanes)

        def conv_inv(j, kvds):
            fiv = fi[...]
            for i in range(2):
                y = _dot(fiv, Yb[i].astype(bf16)) + kvds[i]
                ybuf[pl.ds(j * TM + i * PB, PB), :] = y.astype(bf16)

        def rows_of(p):
            if isinstance(p, int):
                return p % T, pl.ds((p % T) * TM, TM), p % 4
            j = lax.rem(p, T)
            return j, pl.ds(pl.multiple_of(j * TM, TM), TM), lax.rem(p, 4)

        def p_norm(p, x, trigs):
            _, rows, sl = rows_of(p)
            if trigs[0] is not None:
                col = jnp.where(never, jnp.concatenate(trigs, axis=0), x[:, :128])
                x = jnp.concatenate([col, x[:, 128:]], axis=1)
            xa = x + _ln(x) * ybuf[rows, :].astype(f32)
            xin = _ln(xa)
            tt = _ln(xin).astype(bf16)
            xab[sl] = xa + xin
            xinb[sl] = xin
            return tt

        def p_mm(p, tt):
            j, _, _ = rows_of(p)
            pre = _dot(tt, w1[...])
            h = _gelu(pre)
            me = j + 1
            for g, sh in enumerate(SHIFTS):
                ls = slice(g * C4, (g + 1) * C4)
                hg = h[:, ls]
                if sh > 0:
                    hs3[me, sh:TM, ls] = hg[0:TM - sh]
                    hs3[me + 1, 0:sh, ls] = hg[TM - sh:TM]
                else:
                    hs3[me, 0:TM + sh, ls] = hg[-sh:TM]
                    hs3[me - 1, TM + sh:TM, ls] = hg[0:-sh]
            return pre

        def stage_r(p):
            j, rows, sl = rows_of(p)
            hs = _dot(hs3[j + 1].astype(bf16), w2[...])
            x1 = xinb[sl] + hs
            zbuf[rows, :] = _ln(x1).astype(bf16)
            baseb[rows, :] = xab[sl] + hs
            return hs

        def stage_m(p):
            _, rows, _ = rows_of(p)
            zv = zbuf[rows, :]
            acc = baseb[rows, :]
            for c in range(NFC):
                hh = _gelu(_dot(zv, w3[:, c * FC:(c + 1) * FC])).astype(bf16)
                acc = acc + _dot(hh, w4[c * FC:(c + 1) * FC, :])
            return acc

        def step_a(t):
            c = t if t < T else None
            p = t - 1 if 0 <= t - 1 < T else None
            r = t - 3 if t - 3 >= 0 else None
            srcs = []
            if c is not None:
                srcs += conv_fwd_h(c)
            if r is not None:
                srcs += _pieces(stage_r(r), 0, nr_hi)
            ntask = (16 if c is not None else 0) + (32 if p is not None else 0)
            trigs = _pick(srcs, ntask)
            if c is not None and p is not None:
                tk = trigs[0::3]
                tp = [x for i, x in enumerate(trigs) if i % 3]
            else:
                tk = tp = trigs
            srcs = []
            if c is not None:
                us, kvds = conv_kv(c, tk)
            if p is not None:
                tt = p_norm(p, qb[pl.ds(p * TM, TM), :].astype(f32), tp)
            if c is not None:
                conv_fwd_u(c, us)
            if p is not None:
                srcs += _pieces(p_mm(p, tt), 0, np_hi)
            if c is not None:
                conv_mac(c, _pick(srcs, n_mac_tasks))
                conv_inv(c, kvds)

        def body_mrp(s, carry):
            x = stage_m(s)
            hs = stage_r(s + T - 2)
            trigs = []
            for k in range(32):
                n, rr = k // trig_b, (k % trig_b) * (32 // trig_b)
                trigs.append(hs[rr * 8:(rr + 1) * 8, n * 128:(n + 1) * 128])
            p_mm(s + T, p_norm(s + T, x, trigs))
            return carry

        def body_mr(s, carry):
            _, rows, _ = rows_of(s)
            obuf[rows, :] = stage_m(s).astype(bf16)
            stage_r(s + T - 2)
            out_copy(s - T).start()
            return carry

        def body_m(s, carry):
            _, rows, _ = rows_of(s)
            obuf[rows, :] = stage_m(s).astype(bf16)
            out_copy(s - T).start()
            return carry

        if only is not None:
            @pl.when(z == 0)
            def _():
                if isinstance(only, int):
                    step_a(only)
                else:
                    dict(mrp=body_mrp, mr=body_mr, m=body_m)[only](z + T, 0)
            zz = pl.ds(z16, 16)
            obuf[0:16, :] = (ybuf[zz, :] + zbuf[zz, :] + Yb[z, zz, :].astype(bf16)
                             + (baseb[zz, :] + hs3[z, zz, :] + U[z, zz, :] + G[z, zz, :] + hprev[zz, :]
                                + xab[z, zz, :] + xinb[z, zz, :]).astype(bf16))
            out_copy(0).start()
            out_copy(0).wait()
            return

        prologue()
        for t in range(T + 1):
            if t < T:
                for c in in_copies(t)[:3]:
                    c.wait()
            if t >= 1:
                in_copies(t - 1)[3].wait()
            if t == 1:
                w_copies[0].wait()
            if t == 3:
                w_copies[1].wait()
            step_a(t)
            if t + 2 < T:
                for c in in_copies(t + 2):
                    c.start()
            if t == 0:
                w_copies[1].start()
                w_copies[2].start()
            if t == 1:
                w_copies[3].start()
        w_copies[2].wait()
        w_copies[3].wait()
        lax.fori_loop(0, T, body_mrp, 0)
        lax.fori_loop(T, T + 2, body_mr, 0)
        lax.fori_loop(T + 2, 2 * T, body_m, 0)
        for j in range(T):
            out_copy(j).wait()

    @jax.jit
    def fn(A_q, A_k, A_v, A_shift_k, A_ssm_k, A_ssm_D, B_x, B_w1, B_w2, B_w3, B_w4):
        any_spec = pl.BlockSpec(memory_space=pl.ANY)
        scratch = [
            pltpu.VMEM((S, D), bf16),
            pltpu.VMEM((2, TM, D), bf16),
            pltpu.VMEM((2, TM, D), bf16),
            pltpu.VMEM((2, D, TM), bf16),
            pltpu.VMEM((D, D), bf16),
            pltpu.VMEM((D, D), bf16),
            pltpu.VMEM((D, F), bf16),
            pltpu.VMEM((F, D), bf16),
            pltpu.VMEM((D, 4), bf16),
            pltpu.VMEM((1, D), bf16),
            pltpu.VMEM((2 * PB, PB), bf16),
            pltpu.VMEM((PB, 2 * PB), bf16),
            pltpu.VMEM((16, D), f32),
            pltpu.VMEM((8, D), f32),
            pltpu.VMEM((2 * PB, D), f32),
            pltpu.VMEM((NB, 2 * PB, D), f32),
            pltpu.VMEM((NB, 3 * PB, D), f32),
            pltpu.VMEM((2, 2 * PB, D), bf16 if mac_rows % 16 == 0 else f32),
            pltpu.VMEM((S, D), bf16),
            pltpu.VMEM((T + 2, TM, D), f32),
            pltpu.VMEM((4, TM, D), f32),
            pltpu.VMEM((4, TM, D), f32),
            pltpu.VMEM((S, D), f32),
            pltpu.VMEM((S, D), bf16),
            pltpu.VMEM((S, D), bf16),
            pltpu.SemaphoreType.DMA((4, T)),
            pltpu.SemaphoreType.DMA((6,)),
            pltpu.SemaphoreType.DMA((T,)),
        ]
        return pl.pallas_call(
            kernel,
            in_specs=[any_spec] * 10,
            out_specs=any_spec,
            out_shape=jax.ShapeDtypeStruct((1, S, D), bf16),
            scratch_shapes=scratch,
            compiler_params=pltpu.CompilerParams(vmem_limit_bytes=124 * 1024 * 1024),
        )(A_q, A_k, A_v, A_shift_k, A_ssm_k, A_ssm_D.reshape(1, D), B_w1, B_w2, B_w3, B_w4)

    return fn


_impl = make()


@jax.jit
def pallas_interleave_layers__ssm_conv_h3__mixer_s_mlp__prompt_kernel(
        A_q, A_k, A_v, A_shift_k, A_ssm_k, A_ssm_D, B_x, B_w1, B_w2, B_w3, B_w4):
    return _impl(A_q, A_k, A_v, A_shift_k, A_ssm_k, A_ssm_D, B_x, B_w1, B_w2, B_w3, B_w4)
```

```python
import functools
import math

import jax
import jax.numpy as jnp
from jax import lax
import jax.experimental.pallas as pl
import jax.experimental.pallas.tpu as pltpu

S = 2048
D = 1024
F = 3584
TM = 256
T = S // TM
PB = 128
NB = S // PB
C4 = D // 4
EPS = 1e-5
SHIFTS = (1, -1, 2, -2)
NIN = 4
f32 = jnp.float32
bf16 = jnp.bfloat16


def _ln(x):
    m = jnp.mean(x, axis=-1, keepdims=True)
    xc = x - m
    v = jnp.mean(xc * xc, axis=-1, keepdims=True)
    return xc * lax.rsqrt(v + EPS)


def _gelu(x):
    c = math.sqrt(2.0 / math.pi)
    inner = x * (c + (c * 0.044715) * (x * x))
    hx = 0.5 * x
    return hx + hx * jnp.tanh(inner)


def _dot(a, b):
    return jnp.dot(a, b, preferred_element_type=f32)


def _dot_nt(a, b):
    return lax.dot_general(a, b, (((1,), (1,)), ((), ())), preferred_element_type=f32)


def _dft_angle(r, t):
    rr = r & 127
    fr = jnp.where(rr < 64, 2 * rr, 2 * rr - 127)
    m = ((2 * fr + 1) * t + jnp.where(r >= 128, 128, 0)) & 511
    return m.astype(f32) * (2.0 * math.pi / 512.0)


def _pieces(val, ngroup=1):
    rows, cols = val.shape
    out = []
    for n0 in range(0, cols // 128, ngroup):
        for r in range(rows // 8):
            out.append(functools.partial(
                lambda r, n0: val[r * 8:(r + 1) * 8, n0 * 128:(n0 + 1) * 128], r, n0))
    return out


def _run(tasks):
    return [task() for task in tasks]


def _interleave(*lists):
    items = []
    for li, l in enumerate(lists):
        for i, x in enumerate(l):
            items.append(((i + 0.5) / len(l), li, x))
    items.sort(key=lambda e: (e[0], e[1]))
    return [e[2] for e in items]


def _split(tasks, n):
    return [tasks[(i * len(tasks)) // n:((i + 1) * len(tasks)) // n] for i in range(n)]


def make(FC=512, only=None, NA=5, skip_a=False, nrep=None,
         a_kvlo=0.5, a_macrate=2.4, chain_back=32, mc_unroll=True, fence_ug=True, nfence=32, plain=3, a_ord='kl', a_chain=True, fence_y=True, fence=True, mchain=False, mac_dl=False, scopes=False, first=99):
    NFC = F // FC

    def kernel(q_hbm, k_hbm, v_hbm, sk_hbm, hk_hbm, dv_hbm, w1_hbm, w2_hbm, w3_hbm, w4_hbm,
               o_hbm,
               qb, kb, vb, hkb, w1, w2, w3, w4, sk_ref, dv_ref, ff, fi, skt, kcar, hprev, U, G, Yb,
               xb, ybuf, hs3, xab, xinb, zbuf, obuf, ubuf, kvdb,
               sems):
        def is_static(j):
            return isinstance(j, int)

        def rows_at(r0, n):
            return pl.ds(r0 if is_static(r0) else pl.multiple_of(r0, n), n)

        def rem(j, n):
            return j % n if is_static(j) else lax.rem(j, n)

        def in_copy(i, j):
            rows = rows_at(j * TM, TM)
            sl = rem(j, NIN)
            src, dst = [(hk_hbm.at[:, rows], hkb.at[sl]), (k_hbm.at[0, rows, :], kb.at[sl]),
                        (v_hbm.at[0, rows, :], vb.at[sl]), (q_hbm.at[0, rows, :], qb.at[rows, :])][i]
            return pltpu.make_async_copy(src, dst, sems.at[i * T + j])

        def w_copy(i):
            src, dst = [(w1_hbm, w1), (w2_hbm, w2), (sk_hbm, sk_ref), (dv_hbm, dv_ref)][i]
            return pltpu.make_async_copy(src, dst, sems.at[4 * T + i])

        def w34_copies(c):
            cs = pl.ds(c * FC, FC)
            return [pltpu.make_async_copy(w3_hbm.at[:, cs], w3.at[:, cs], sems.at[4 * T + 4 + 2 * c]),
                    pltpu.make_async_copy(w4_hbm.at[cs, :], w4.at[cs, :], sems.at[4 * T + 5 + 2 * c])]

        def out_copy(j):
            rows = rows_at(j * TM, TM)
            return pltpu.make_async_copy(obuf.at[rows, :], o_hbm.at[0, rows, :], sems.at[4 * T + 4 + 2 * NFC + j])

        z = jnp.min(lax.broadcasted_iota(jnp.int32, (8, 128), 1))
        never = z > 0
        z16 = pl.multiple_of(z, 16)
        zs = 0 if fence else z16
        zl = z16 if fence else 0
        ZERO = jnp.zeros((8, 128), f32)

        def need(w, dls, lo=0.0, hi=1.0):
            dls = [d for d in dls if d is not None]
            if not dls:
                return w
            nt = w.shape[1] // 128
            cols = [w[:, n * 128:(n + 1) * 128] for n in range(nt)]
            npass = w.shape[0] // 512
            slots = nt * npass
            for i, d in enumerate(dls):
                sidx = min(slots - 1, int((lo + (hi - lo) * (i + 1) / len(dls)) * slots - 1e-6))
                n, r0 = sidx // npass, (sidx % npass) * 512
                col = cols[n]
                parts = [col[:r0]] if r0 else []
                parts += [jnp.where(never, d, col[r0:r0 + 16]), col[r0 + 16:]]
                cols[n] = jnp.concatenate(parts, axis=0)
            return jnp.concatenate(cols, axis=1)

        def after(x, srcs):
            if not srcs:
                return x
            d = srcs[max(0, len(srcs) - 1 - chain_back)]()
            d = jnp.concatenate([d, d], axis=0).astype(bf16)
            head = jnp.where(never, d, x[:16, :128])
            if x.shape[1] > 128:
                head = jnp.concatenate([head, x[:16, 128:]], axis=1)
            return jnp.concatenate([head, x[16:]], axis=0)

        def release(srcs, q=False, k=False, x1=False, x=False, n=32):
            for kk in range(n):
                d = srcs[kk % len(srcs)]()
                ls = slice((kk % 8) * 128, (kk % 8 + 1) * 128)
                g = kk // 8
                if q or k:
                    d2 = jnp.concatenate([d, d], axis=0).astype(bf16)
                if q:
                    qb[pl.ds(pl.multiple_of(z + S + 16 * g, 16), 16), ls] = d2
                if k:
                    kb[z + NIN, 16 * g:16 * g + 16, ls] = d2
                if x1:
                    xinb[z + 4, 8 * g:8 * g + 8, ls] = d
                if x:
                    xb[pl.ds(pl.multiple_of(z + S + 8 * g, 8), 8), ls] = d

        def constants():
            r = lax.broadcasted_iota(jnp.int32, (2 * PB, PB), 0)
            t = lax.broadcasted_iota(jnp.int32, (2 * PB, PB), 1)
            ff[...] = jnp.cos(_dft_angle(r, t)).astype(bf16)
            r = lax.broadcasted_iota(jnp.int32, (PB, 2 * PB), 1)
            t = lax.broadcasted_iota(jnp.int32, (PB, 2 * PB), 0)
            fi[...] = (jnp.cos(_dft_angle(r, t)) * (1.0 / PB)).astype(bf16)
            kcar[...] = jnp.zeros((8, D), f32)
            hs3[1, 0:8, :] = jnp.zeros((8, D), f32)
            hs3[T, TM - 8:TM, :] = jnp.zeros((8, D), f32)
            if not mc_unroll:
                G[NB] = jnp.zeros((3 * PB, D), f32)

        def job_h(j, prev=()):
            sl = rem(j, NIN)
            ffv = after(ff[...], prev)
            srcs = []
            hlast = None
            for i in range(2):
                hh = _dot_nt(ffv, hkb[sl, :, i * PB:(i + 1) * PB])
                srcs += _pieces(hh, 4)
                gr, gi = hh[:PB], hh[PB:]
                if not (is_static(j) and j == 0 and i == 0):
                    hp = hprev[...] if i == 0 else hlast
                    pr, pi_ = hp[:PB], hp[PB:]
                    gr = jnp.concatenate([gr[:64] - pi_[:64], gr[64:] + pi_[64:]], axis=0)
                    gi = jnp.concatenate([gi[:64] + pr[:64], gi[64:] - pr[64:]], axis=0)
                b = (0 if fence_ug else z) + 2 * j + i
                G[b, 0:PB, :] = gr
                G[b, PB:2 * PB, :] = gi - gr
                G[b, 2 * PB:3 * PB, :] = gr + gi
                hlast = hh
            hprev[...] = hlast
            if fence_ug:
                for kk in range(nfence):
                    G[z + NB, 8 * (kk % 32):8 * (kk % 32) + 8, (kk // 32) * 128:(kk // 32 + 1) * 128] = srcs[max(0, len(srcs) - nfence + kk)]()
            return srcs

        def tasks_kv(j, with_x):
            sl = rem(j, NIN)

            def task(i, lt):
                ls = slice(lt * 128, (lt + 1) * 128)
                rs = slice(i * PB, (i + 1) * PB)
                kf = kb[sl, rs, ls].astype(f32)
                if i == 0:
                    prev = kcar[:, ls]
                else:
                    prev = kb[sl, PB - 16:PB, ls].astype(f32)[8:]
                    kcar[:, ls] = kf[PB - 8:]
                ext = jnp.concatenate([prev, kf], axis=0)
                ks = kf * skt[0:1, ls]
                for tt in range(1, 4):
                    ks = ks + ext[8 - tt:8 - tt + PB, :] * skt[tt:tt + 1, ls]
                kv = ks * vb[sl, rs, ls].astype(f32)
                ubuf[pl.ds(zs + i * PB, PB), ls] = kv.astype(bf16)
                kvdb[pl.ds(zs + i * PB, PB), ls] = kv * skt[4:5, ls]
                done = kvdb[pl.ds(zl, 16), 0:128]
                if with_x:
                    xrows = rows_at(j * TM + i * PB, PB)
                    xb[xrows, ls] = qb[xrows, ls].astype(f32)
                    done = done + xb[pl.ds(z16, 16), 0:128]
                return jnp.where(never, ubuf[pl.ds(zl, 16), 0:128], done.astype(bf16))

            return [functools.partial(task, i, lt) for i in range(2) for lt in range(8)]

        def job_u(j, prev=()):
            if fence:
                ubuf[pl.ds(z16 + TM, 16), 0:128] = jnp.zeros((16, 128), bf16)
                kvdb[pl.ds(z16 + TM, 8), 0:128] = ZERO
            ffv = after(ff[...], prev)
            srcs = []
            for i in range(2):
                uu = _dot(ffv, ubuf[i * PB:(i + 1) * PB, :])
                srcs += _pieces(uu, 4)
                U[(0 if fence_ug else z) + 2 * j + i] = uu
            if fence_ug:
                for kk in range(nfence):
                    U[z + NB, 8 * (kk % 32):8 * (kk % 32) + 8, (kk // 32) * 128:(kk // 32 + 1) * 128] = srcs[max(0, len(srcs) - nfence + kk)]()
            return srcs

        def tasks_mac(j):
            RG, LG = 16, 256
            if is_static(j):
                nterm = 2 * j + 2
                uidx = list(range(nterm))
                gidx = [2 * j + 1 - b for b in range(nterm)]
            else:
                nterm = NB
                uidx = [jnp.where(b <= 2 * j + 1, b, 0) for b in range(nterm)]
                gidx = [jnp.where(b <= 2 * j + 1, 2 * j + 1 - b, NB) for b in range(nterm)]

            def task(r0, l0):
                ls = slice(l0, l0 + LG)

                def ld(ref, idx, p):
                    return ref[idx, p * PB + r0:p * PB + r0 + RG, ls]

                acc1 = acc2 = None
                g2 = [ld(G, gidx[0], p) for p in range(3)]
                for b in range(nterm):
                    ua, ub = ld(U, uidx[b], 0), ld(U, uidx[b], 1)
                    us = ua + ub
                    t2 = [g2[0] * us, g2[1] * ua, g2[2] * ub]
                    acc2 = t2 if b == 0 else [x + y for x, y in zip(acc2, t2)]
                    if b < nterm - 1:
                        g2 = [ld(G, gidx[b + 1], p) for p in range(3)]
                        t1 = [g2[0] * us, g2[1] * ua, g2[2] * ub]
                        acc1 = t1 if b == 0 else [x + y for x, y in zip(acc1, t1)]
                for i, acc in enumerate((acc1, acc2)):
                    zy = 0 if fence_y else z16
                    Yb[i, pl.ds(zy + r0, RG), ls] = (acc[0] - acc[2]).astype(bf16)
                    Yb[i, pl.ds(zy + PB + r0, RG), ls] = (acc[0] + acc[1]).astype(bf16)
                return Yb[z if fence_y else 0, 0:16, 0:128]

            return [functools.partial(task, r0, l0) for r0 in range(0, PB, RG) for l0 in range(0, D, LG)]

        def job_inv(j, prev=()):
            if fence_y:
                Yb[z + 2, 0:16, 0:128] = jnp.zeros((16, 128), bf16)
            fiv = after(fi[...], prev)
            srcs = []
            for i in range(2):
                yc = _dot(fiv, Yb[i])
                srcs += _pieces(yc, 2)
                y = yc + kvdb[i * PB:(i + 1) * PB, :]
                ybuf[rows_at(j * TM + i * PB, PB), :] = y.astype(bf16)
            return srcs

        def tasks_ln(p, res, from_q=False, with_dl=True):
            j = rem(p, T)
            s3, s4 = rem(p, 3), rem(p, 4)
            res['t'] = [None] * 16

            def task(k):
                rows = rows_at(j * TM + k * 16, 16)
                x = qb[rows, :].astype(f32) if from_q else xb[rows, :]
                xa = x + _ln(x) * ybuf[rows, :].astype(f32)
                xin = _ln(xa)
                res['t'][k] = _ln(xin).astype(bf16)
                xab[s3, k * 16:(k + 1) * 16, :] = xa + xin
                xinb[s4, k * 16:(k + 1) * 16, :] = xin
                if not with_dl:
                    return None
                done = (xab[z + s3, 0:16, 0:128] + xinb[z + s4, 0:16, 0:128]).astype(bf16)
                return jnp.where(never, res['t'][k][:, 0:128], done)

            return [functools.partial(task, k) for k in range(16)]

        def tasks_ln2(p):
            j = rem(p, T)
            s4 = rem(p, 4)

            def task(k):
                rows = rows_at(j * TM + k * 16, 16)
                zbuf[rows, :] = _ln(xinb[s4, k * 16:(k + 1) * 16, :]).astype(bf16)
                return zbuf[rows_at(z + 0, 16), 0:128]

            return [functools.partial(task, k) for k in range(16)]

        def job_w1(p, res, prev=(), dls=()):
            j = rem(p, T)
            pre = _dot(after(jnp.concatenate(res['t'], axis=0), prev), need(w1[...], dls, 0.1))
            h = _gelu(pre)
            me = j + 1
            for g, sh in enumerate(SHIFTS):
                ls = slice(g * C4, (g + 1) * C4)
                hg = h[:, ls]
                if sh > 0:
                    hs3[me, sh:TM, ls] = hg[0:TM - sh]
                    hs3[me + 1, 0:sh, ls] = hg[TM - sh:TM]
                else:
                    hs3[me, 0:TM + sh, ls] = hg[-sh:TM]
                    hs3[me - 1, TM + sh:TM, ls] = hg[0:-sh]
            return _pieces(pre)

        def job_w2(p, dls=(), prev=(), lo=0.0):
            j = rem(p, T)
            s3, s4 = rem(p, 3), rem(p, 4)
            hs = _dot(after(hs3[j + 1].astype(bf16), prev), need(w2[...], dls, lo))
            xinb[s4] = xinb[s4] + hs
            xb[rows_at(j * TM, TM), :] = xab[s3] + hs
            return _pieces(hs)

        def m_begin(p):
            rows = rows_at(rem(p, T) * TM, TM)
            return dict(rows=rows, z=zbuf[rows, :], acc=xb[rows, :])

        def job_m(st, c, t3=(), t4=()):
            zin = after(st['z'], st.pop('prev', st.get('last', ()))) if mchain else st['z']
            pre = _dot(zin, need(w3[:, c * FC:(c + 1) * FC], st.pop('dl', [])))
            hh = _gelu(pre).astype(bf16)
            part = _dot(hh, need(w4[c * FC:(c + 1) * FC, :], _run(t3)))
            st['acc'] = st['acc'] + part
            st['dl'] = _run(t4)
            st['last'] = _pieces(part)

        def m_end(st, to_x, to_o):
            if to_x:
                xb[st['rows'], :] = st['acc']
            if to_o:
                obuf[st['rows'], :] = st['acc'].astype(bf16)

        def m_jobs(st, tasks, c0=0):
            n = 2 * (NFC - c0) - 1
            parts = _split(tasks, n) + [[]]
            for c in range(c0, NFC):
                job_m(st, c, parts[2 * (c - c0)], parts[2 * (c - c0) + 1])

        def step_a(t):
            c, p, r = t, t - 1, t - 3
            res = {}
            if plain == 3:
                d2 = _run(tasks_ln2(r - 1)) if r >= 1 else []
                prev = job_w2(r, d2[3::4], lo=a_kvlo) if r >= 0 else job_h(c)
                release(prev, q=p >= 0, k=True)
                tasks = dict(k=tasks_kv(c, t == NA - 1),
                             l=tasks_ln(p, res, from_q=True, with_dl=False) if p >= 0 else [])
                for key in a_ord:
                    _run(tasks[key])
                if r >= 0:
                    prev = job_h(c, prev if a_chain else ())
                prev = job_u(c, prev if a_chain else ())
                dm = _run(tasks_mac(c))
                if p >= 0:
                    nd = min(len(dm), int(a_macrate * 4096 / (26 * (4 * c + 3))))
                    prev = job_w1(p, res, prev if a_chain else (), dm[:nd])
                job_inv(c, prev if a_chain else ())
                return
            if plain:
                ch = (lambda x: x) if plain == 2 else (lambda x: ())
                prev = ()
                if r >= 1:
                    _run(tasks_ln2(r - 1))
                _run(tasks_kv(c, t == NA - 1))
                if p >= 0:
                    _run(tasks_ln(p, res, from_q=True, with_dl=False))
                if r >= 0:
                    prev = job_w2(r)
                prev = job_h(c, ch(prev))
                prev = job_u(c, ch(prev))
                _run(tasks_mac(c))
                if p >= 0:
                    prev = job_w1(p, res, ch(prev))
                job_inv(c, ch(prev))
                return
            dk = _run(tasks_kv(c, t == NA - 1))
            if r >= 0:
                if r >= 1:
                    dk = _interleave(dk, _run(tasks_ln2(r - 1)))
                prev = job_w2(r, dk, lo=a_kvlo)
            else:
                prev = job_h(c)
            if p >= 0:
                d = prev[0]()
                qb[pl.ds(pl.multiple_of(z + S, 16), 16), 0:128] = jnp.concatenate([d, d], axis=0).astype(bf16)
                _run(tasks_ln(p, res, from_q=True, with_dl=False))
            if r >= 0:
                prev = job_h(c, prev)
            prev = job_u(c, prev)
            dm = _run(tasks_mac(c))
            if p >= 0:
                nd = min(len(dm), int(a_macrate * 4096 / (26 * (4 * c + 3))))
                prev = job_w1(p, res, prev, dm[:nd])
            job_inv(c, prev)

        def body_mc(t, carry):
            for i in range(4):
                in_copy(i, t).wait()
            res = {}
            st = m_begin(t - NA)
            st['prev'] = job_h(t)
            job_m(st, 0, tasks_kv(t, True))
            st['prev'] = job_u(t, st['last'] if mchain else ())
            if mac_dl:
                m_jobs(st, _interleave(tasks_mac(t), tasks_ln2(t - 4) + tasks_ln(t - 1, res)), 1)
            else:
                _run(tasks_mac(t))
                m_jobs(st, tasks_ln2(t - 4) + tasks_ln(t - 1, res), 1)
            m_end(st, True, False)
            prev = job_inv(t, st['last'] if mchain else ())
            prev = job_w2(t - 3, prev=prev if mchain else ())
            job_w1(t - 1, res, prev=prev if mchain else ())
            return carry

        def body_mpr(t, carry):
            res = {}
            st = m_begin(t - NA)
            m_jobs(st, tasks_ln2(t - 4) + tasks_ln(t - 1, res))
            m_end(st, True, True)
            job_w2(t - 3)
            job_w1(t - 1, res)

            @pl.when(t - NA >= T)
            def _():
                out_copy(t - NA - T).start()
            return carry

        def body_mr(t, carry):
            st = m_begin(t - NA)
            m_jobs(st, tasks_ln2(t - 4))
            m_end(st, False, True)
            job_w2(t - 3)
            out_copy(t - NA - T).start()
            return carry

        def body_m(t, carry):
            st = m_begin(t - NA)
            m_jobs(st, tasks_ln2(jnp.minimum(t - 4, 2 * T - 1)))
            m_end(st, False, True)
            out_copy(t - NA - T).start()
            return carry

        if only is not None:
            @pl.when(z == 0)
            def _():
                if isinstance(only, int):
                    step_a(only) if only < NA else body_mc(only, 0)
                else:
                    dict(mc=body_mc, mpr=body_mpr, mr=body_mr, m=body_m)[only](z + (NA if only == 'mc' else NA + T), 0)
            zz = pl.ds(z16, 16)
            obuf[0:16, :] = (ybuf[zz, :] + zbuf[zz, :] + Yb[z, zz, :]
                             + (hs3[z, zz, :] + U[z, zz, :] + G[z, zz, :] + hprev[zz, :]
                                + xab[z, zz, :] + xinb[z, zz, :] + xb[zz, :]).astype(bf16))
            out_copy(0).start()
            out_copy(0).wait()
            return

        import contextlib
        scope = jax.named_scope if scopes else (lambda name: contextlib.nullcontext())

        def tile(j, qs=()):
            return [in_copy(i, j) for i in range(3)] + [in_copy(3, x) for x in qs]

        def chunks(lo, hi):
            return [cp for c in range(lo, hi) for cp in w34_copies(c)]

        issue = {
            0: [w_copy(2), w_copy(3)] + tile(0) + tile(1, [0]) + [w_copy(0)] + tile(2, [1]) + tile(3, [2])
               + [w_copy(1)],
            1: chunks(0, 3) + tile(4, [3, 4]),
            2: chunks(3, NFC) + tile(5, [5]),
            3: tile(6, [6]),
            4: tile(7, [7]),
        }
        for cp in issue[0][:first]:
            cp.start()
        with scope("const"):
            constants()
        w_copy(2).wait()
        w_copy(3).wait()
        skt[0:4, :] = sk_ref[...].astype(f32)
        skt[4:8, :] = jnp.broadcast_to(dv_ref[...].astype(f32).reshape(1, D), (4, D))
        for cp in issue[0][first:]:
            cp.start()
        for t in range(NA):
            if t > 0:
                for cp in issue[t]:
                    cp.start()
            with scope(f"wait{t}"):
                for i in range(3):
                    in_copy(i, t).wait()
                if t >= 1:
                    in_copy(3, t - 1).wait()
                if t == NA - 1:
                    in_copy(3, t).wait()
                if t == 1:
                    w_copy(0).wait()
                if t == 3:
                    w_copy(1).wait()

            with scope(f"stepA{t}"):
                @pl.when(z == 0)
                def _(t=t):
                    if not skip_a:
                        step_a(t)
        with scope("waitW"):
            for cp in chunks(0, NFC):
                cp.wait()
        if nrep is not None:
            nmc, nmpr = nrep
            if nmc:
                lax.fori_loop(NA, NA + nmc, body_mc, 0)
            for t in range(NA + nmc, T):
                for i in range(4):
                    in_copy(i, t).wait()
            if nmpr:
                lax.fori_loop(T, T + nmpr, body_mpr, 0)
            out_copy(0).start()
            out_copy(0).wait()
            return
        if mc_unroll:
            for t in range(NA, T):
                with scope(f"MC{t}"):
                    @pl.when(z == 0)
                    def _(t=t):
                        body_mc(t, 0)
        else:
            with scope("loopMC"):
                lax.fori_loop(NA, T, body_mc, 0)
        with scope("loopMPR"):
            lax.fori_loop(T, 2 * T + 1, body_mpr, 0)
        with scope("loopMR"):
            lax.fori_loop(2 * T + 1, 2 * T + 3, body_mr, 0)
        with scope("loopM"):
            lax.fori_loop(2 * T + 3, 2 * T + NA, body_m, 0)
        with scope("waitO"):
            for j in range(T):
                out_copy(j).wait()

    @jax.jit
    def fn(A_q, A_k, A_v, A_shift_k, A_ssm_k, A_ssm_D, B_x, B_w1, B_w2, B_w3, B_w4):
        any_spec = pl.BlockSpec(memory_space=pl.ANY)
        scratch = [
            pltpu.VMEM((S + 64, D), bf16),
            pltpu.VMEM((NIN + 1, TM, D), bf16),
            pltpu.VMEM((NIN, TM, D), bf16),
            pltpu.VMEM((NIN, D, TM), bf16),
            pltpu.VMEM((D, D), bf16),
            pltpu.VMEM((D, D), bf16),
            pltpu.VMEM((D, F), bf16),
            pltpu.VMEM((F, D), bf16),
            pltpu.VMEM((4, D), bf16),
            pltpu.VMEM((D,), bf16),
            pltpu.VMEM((2 * PB, PB), bf16),
            pltpu.VMEM((PB, 2 * PB), bf16),
            pltpu.VMEM((8, D), f32),
            pltpu.VMEM((8, D), f32),
            pltpu.VMEM((2 * PB, D), f32),
            pltpu.VMEM((NB + 1, 2 * PB, D), f32),
            pltpu.VMEM((NB + 1, 3 * PB, D), f32),
            pltpu.VMEM((3, 2 * PB, D), bf16),
            pltpu.VMEM((S + 32, D), f32),
            pltpu.VMEM((S, D), bf16),
            pltpu.VMEM((T + 2, TM, D), f32),
            pltpu.VMEM((3, TM, D), f32),
            pltpu.VMEM((5, TM, D), f32),
            pltpu.VMEM((S, D), bf16),
            pltpu.VMEM((S, D), bf16),
            pltpu.VMEM((TM + 16, D), bf16),
            pltpu.VMEM((TM + 16, D), f32),
            pltpu.SemaphoreType.DMA((5 * T + 4 + 2 * NFC,)),
        ]
        return pl.pallas_call(
            kernel,
            in_specs=[any_spec] * 10,
            out_specs=any_spec,
            out_shape=jax.ShapeDtypeStruct((1, S, D), bf16),
            scratch_shapes=scratch,
            compiler_params=pltpu.CompilerParams(vmem_limit_bytes=124 * 1024 * 1024),
        )(A_q, A_k, A_v, A_shift_k.T, A_ssm_k, A_ssm_D, B_w1, B_w2, B_w3, B_w4)

    return fn


_impl = make()


@jax.jit
def pallas_interleave_layers__ssm_conv_h3__mixer_s_mlp__prompt_kernel(
        A_q, A_k, A_v, A_shift_k, A_ssm_k, A_ssm_D, B_x, B_w1, B_w2, B_w3, B_w4):
    return _impl(A_q, A_k, A_v, A_shift_k, A_ssm_k, A_ssm_D, B_x, B_w1, B_w2, B_w3, B_w4)
```

```python
import contextlib
import functools
import math

import jax
import jax.numpy as jnp
from jax import lax
import jax.experimental.pallas as pl
import jax.experimental.pallas.tpu as pltpu

S = 2048
D = 1024
F = 3584
TM = 256
T = S // TM
PB = 128
NB = S // PB
C4 = D // 4
EPS = 1e-5
SHIFTS = (1, -1, 2, -2)
NIN = 4
f32 = jnp.float32
bf16 = jnp.bfloat16


def _ln(x):
    m = jnp.mean(x, axis=-1, keepdims=True)
    xc = x - m
    v = jnp.mean(xc * xc, axis=-1, keepdims=True)
    return xc * lax.rsqrt(v + EPS)


def _gelu(x):
    c = math.sqrt(2.0 / math.pi)
    inner = x * (c + (c * 0.044715) * (x * x))
    hx = 0.5 * x
    return hx + hx * jnp.tanh(inner)


def _dot(a, b):
    return jnp.dot(a, b, preferred_element_type=f32)


def _dot_nt(a, b):
    return lax.dot_general(a, b, (((1,), (1,)), ((), ())), preferred_element_type=f32)


def _dft_angle(r, t):
    rr = r & 127
    fr = jnp.where(rr < 64, 2 * rr, 2 * rr - 127)
    m = ((2 * fr + 1) * t + jnp.where(r >= 128, 128, 0)) & 511
    return m.astype(f32) * (2.0 * math.pi / 512.0)


def _pieces(val, ngroup=1):
    rows, cols = val.shape
    out = []
    for n0 in range(0, cols // 128, ngroup):
        for r in range(rows // 8):
            out.append(functools.partial(
                lambda r, n0: val[r * 8:(r + 1) * 8, n0 * 128:(n0 + 1) * 128], r, n0))
    return out


class _Gated:
    def __init__(self, fn):
        self.fn = fn

    def __call__(self, gate=None):
        return self.fn(gate=gate)


def _run(tasks, srcs=None):
    out = []
    for i, task in enumerate(tasks):
        if srcs and isinstance(task, _Gated):
            out.append(task(srcs[(i * len(srcs)) // len(tasks)]()))
        else:
            out.append(task())
    return out


def _interleave(*lists):
    items = []
    for li, l in enumerate(lists):
        for i, x in enumerate(l):
            items.append(((i + 0.5) / len(l), li, x))
    items.sort(key=lambda e: (e[0], e[1]))
    return [e[2] for e in items]


def _split(tasks, n):
    return [tasks[(i * len(tasks)) // n:((i + 1) * len(tasks)) // n] for i in range(n)]


def make(FC=512, only=None, NA=5, skip_a=False, nrep=None,
         a_kvlo=0.5, a_macrate=2.4, chain_back=32, mc_unroll=True, fence_ug=True, nfence=32, plain=3, a_ord='kl', a_chain=True, kv_split=10, chain_hops=0, mac_nd=4, h_after=5, ln_from=3, gates=True, ufence=0, mac_gate=0, mac_gdl=False, mac_slack=1, ln_groups=1, kv_strided=True, fence_y=True, fence=True, mchain=False, mac_dl=False, scopes=False, first=99):
    NFC = F // FC

    def kernel(q_hbm, k_hbm, v_hbm, sk_hbm, hk_hbm, dv_hbm, w1_hbm, w2_hbm, w3_hbm, w4_hbm,
               o_hbm,
               qb, kb, vb, hkb, w1, w2, w3, w4, sk_ref, dv_ref, ff, fi, skt, kcar, hprev, U, G, Yb,
               xb, ybuf, hs3, xab, xinb, zbuf, obuf, ubuf, tbuf, kst, baseb,
               sems):
        def is_static(j):
            return isinstance(j, int)

        def rows_at(r0, n):
            return pl.ds(r0 if is_static(r0) else pl.multiple_of(r0, n), n)

        def rem(j, n):
            return j % n if is_static(j) else lax.rem(j, n)

        def in_copy(i, j):
            rows = rows_at(j * TM, TM)
            sl = rem(j, NIN)
            src, dst = [(hk_hbm.at[:, rows], hkb.at[sl]), (k_hbm.at[0, rows, :], kb.at[sl]),
                        (v_hbm.at[0, rows, :], vb.at[sl]), (q_hbm.at[0, rows, :], qb.at[rows, :])][i]
            return pltpu.make_async_copy(src, dst, sems.at[i * T + j])

        def w_copy(i):
            src, dst = [(w1_hbm, w1), (w2_hbm, w2), (sk_hbm, sk_ref), (dv_hbm, dv_ref)][i]
            return pltpu.make_async_copy(src, dst, sems.at[4 * T + i])

        def w34_copies(c):
            cs = pl.ds(c * FC, FC)
            return [pltpu.make_async_copy(w3_hbm.at[:, cs], w3.at[:, cs], sems.at[4 * T + 4 + 2 * c]),
                    pltpu.make_async_copy(w4_hbm.at[cs, :], w4.at[cs, :], sems.at[4 * T + 5 + 2 * c])]

        def out_copy(j):
            rows = rows_at(j * TM, TM)
            return pltpu.make_async_copy(obuf.at[rows, :], o_hbm.at[0, rows, :], sems.at[4 * T + 4 + 2 * NFC + j])

        z = jnp.min(lax.broadcasted_iota(jnp.int32, (8, 128), 1))
        never = z > 0
        never2 = z > 1
        z16 = pl.multiple_of(z, 16)

        def need(w, dls, lo=0.0, hi=1.0):
            dls = [d for d in dls if d is not None]
            if not dls:
                return w
            nt = w.shape[1] // 128
            cols = [w[:, n * 128:(n + 1) * 128] for n in range(nt)]
            npass = w.shape[0] // 512
            slots = nt * npass
            used = {}
            for i, d in enumerate(dls):
                sidx = min(slots - 1, int((lo + (hi - lo) * (i + 1) / len(dls)) * slots - 1e-6))
                used[sidx] = used.get(sidx, -1) + 1
                n, r0 = sidx // npass, (sidx % npass) * 512 + 16 * used[sidx]
                col = cols[n]
                parts = [col[:r0]] if r0 else []
                parts += [jnp.where(never, d, col[r0:r0 + 16]), col[r0 + 16:]]
                cols[n] = jnp.concatenate(parts, axis=0)
            return jnp.concatenate(cols, axis=1)

        def after(x, srcs):
            if not srcs:
                return x
            d = srcs[max(0, len(srcs) - 1 - chain_back)]()
            for _ in range(chain_hops):
                d = jnp.broadcast_to(jnp.sum(d, axis=-1, keepdims=True), (8, 128))
            d = jnp.concatenate([d, d], axis=0).astype(bf16)
            head = jnp.where(never, d, x[:16, :128])
            if x.shape[1] > 128:
                head = jnp.concatenate([head, x[:16, 128:]], axis=1)
            return jnp.concatenate([head, x[16:]], axis=0)

        def release(srcs, q=False, k=False, x1=False, x=False, n=32):
            for kk in range(n):
                d = srcs[kk % len(srcs)]()
                ls = slice((kk % 8) * 128, (kk % 8 + 1) * 128)
                g = kk // 8
                if q or k:
                    d2 = jnp.concatenate([d, d], axis=0).astype(bf16)
                if q:
                    qb[pl.ds(pl.multiple_of(z + S + 16 * g, 16), 16), ls] = d2
                if k:
                    kb[z + NIN, 16 * g:16 * g + 16, ls] = d2
                if x1:
                    xinb[z + 4, 8 * g:8 * g + 8, ls] = d
                if x:
                    xb[pl.ds(pl.multiple_of(z + S + 8 * g, 8), 8), ls] = d

        def constants():
            r = lax.broadcasted_iota(jnp.int32, (2 * PB, PB), 0)
            t = lax.broadcasted_iota(jnp.int32, (2 * PB, PB), 1)
            ff[...] = jnp.cos(_dft_angle(r, t)).astype(bf16)
            r = lax.broadcasted_iota(jnp.int32, (PB, 2 * PB), 1)
            t = lax.broadcasted_iota(jnp.int32, (PB, 2 * PB), 0)
            fi[...] = (jnp.cos(_dft_angle(r, t)) * (1.0 / PB)).astype(bf16)
            kcar[...] = jnp.zeros((8, D), f32)
            kst[:, 0:16, :] = jnp.zeros((4, 16, 128), f32)
            hs3[1, 0:8, :] = jnp.zeros((8, D), f32)
            hs3[T, TM - 8:TM, :] = jnp.zeros((8, D), f32)
            if not mc_unroll:
                G[NB] = jnp.zeros((3 * PB, D), f32)

        def job_h(j, prev=(), g_fence=False):
            sl = rem(j, NIN)
            ffv = after(ff[...], prev)
            srcs = []
            hlast = None
            for i in range(2):
                hh = _dot_nt(ffv, hkb[sl, :, i * PB:(i + 1) * PB])
                srcs += _pieces(hh, 4)
                gr, gi = hh[:PB], hh[PB:]
                if not (is_static(j) and j == 0 and i == 0):
                    hp = hprev[...] if i == 0 else hlast
                    pr, pi_ = hp[:PB], hp[PB:]
                    gr = jnp.concatenate([gr[:64] - pi_[:64], gr[64:] + pi_[64:]], axis=0)
                    gi = jnp.concatenate([gi[:64] + pr[:64], gi[64:] - pr[64:]], axis=0)
                b = 2 * j + i
                G[b, 0:PB, :] = gr
                G[b, PB:2 * PB, :] = gi - gr
                G[b, 2 * PB:3 * PB, :] = gr + gi
                hlast = hh
            hprev[...] = hlast
            if g_fence:
                for kk in range(nfence):
                    G[z + NB, 8 * (kk % 32):8 * (kk % 32) + 8, 0:128] = srcs[max(0, len(srcs) - nfence + kk)]()
            return srcs

        def tasks_kv(j, with_x):
            sl = rem(j, NIN)

            def task(i, lt):
                ls = slice(lt * 128, (lt + 1) * 128)
                rs = slice(i * PB, (i + 1) * PB)
                kf = kb[sl, rs, ls].astype(f32)
                if kv_strided:
                    pair, par = lt // 2, lt % 2
                    kst[pair, pl.ds(2 * (8 + i * PB) + par, PB, stride=2), :] = kf
                    ks = kf * skt[0:1, ls]
                    for tt in range(1, 4):
                        ks = ks + kst[pair, pl.ds(2 * (8 - tt + i * PB) + par, PB, stride=2), :] * skt[tt:tt + 1, ls]
                    if i == 1:
                        kst[pair, pl.ds(par, 8, stride=2), :] = kf[PB - 8:]
                else:
                    if i == 0:
                        prev = kcar[:, ls]
                    else:
                        prev = kb[sl, PB - 16:PB, ls].astype(f32)[8:]
                        kcar[:, ls] = kf[PB - 8:]
                    ext = jnp.concatenate([prev, kf], axis=0)
                    ks = kf * skt[0:1, ls]
                    for tt in range(1, 4):
                        ks = ks + ext[8 - tt:8 - tt + PB, :] * skt[tt:tt + 1, ls]
                kv = ks * vb[sl, rs, ls].astype(f32)
                ubuf[i * PB:(i + 1) * PB, ls] = kv.astype(bf16)
                done = ubuf[pl.ds(z16 + i * PB, 16), ls]
                if with_x:
                    xrows = rows_at(j * TM + i * PB, PB)
                    xb[xrows, ls] = qb[xrows, ls].astype(f32)
                    done = jnp.where(never2, xb[pl.ds(z16, 16), ls].astype(bf16), done)
                return done

            return [functools.partial(task, i, lt) for i in range(2) for lt in range(8)]

        def job_u(j, prev=(), fence=True):
            ubuf[pl.ds(z16 + TM, 16), 0:128] = jnp.zeros((16, 128), bf16)
            ffv = after(ff[...], prev)
            srcs = []
            for i in range(2):
                uu = _dot(ffv, ubuf[i * PB:(i + 1) * PB, :])
                srcs += _pieces(uu, 4)
                U[2 * j + i] = uu
            if fence and ufence == 1:
                U[z + NB, pl.ds(pl.multiple_of(z, 8), 8), pl.ds(pl.multiple_of(z, 128), 128)] = srcs[-1]()
            elif fence and ufence == 2:
                U[NB, pl.ds(pl.multiple_of(z, 8), 8), 0:128] = srcs[-1]()
            elif fence:
                for kk in range(nfence):
                    U[z + NB, 8 * (kk % 32):8 * (kk % 32) + 8, (kk // 32) * 128:(kk // 32 + 1) * 128] = srcs[max(0, len(srcs) - nfence + kk)]()
            return srcs

        def tasks_mac(j, LG=256):
            RG = 16
            if is_static(j):
                nterm = 2 * j + 2
                uidx = list(range(nterm))
                gidx = [2 * j + 1 - b for b in range(nterm)]
            else:
                nterm = NB
                uidx = [jnp.where(b <= 2 * j + 1, b, 0) for b in range(nterm)]
                gidx = [jnp.where(b <= 2 * j + 1, 2 * j + 1 - b, NB) for b in range(nterm)]

            def task(r0, l0, gate=None):
                ls = slice(l0, l0 + LG)
                if gate is not None:
                    gate = jnp.concatenate([gate] * (RG // 8), axis=0)
                    gate = jnp.concatenate([gate] * (LG // 128), axis=1)
                    U[z + NB, r0:r0 + RG, ls] = gate
                    U[z + NB, PB + r0:PB + r0 + RG, ls] = gate

                def ld(ref, idx, p):
                    return ref[idx, p * PB + r0:p * PB + r0 + RG, ls]

                acc1 = acc2 = None
                g2 = [ld(G, gidx[0], p) for p in range(3)]
                for b in range(nterm):
                    ua, ub = ld(U, uidx[b], 0), ld(U, uidx[b], 1)
                    us = ua + ub
                    t2 = [g2[0] * us, g2[1] * ua, g2[2] * ub]
                    acc2 = t2 if b == 0 else [x + y for x, y in zip(acc2, t2)]
                    if b < nterm - 1:
                        g2 = [ld(G, gidx[b + 1], p) for p in range(3)]
                        t1 = [g2[0] * us, g2[1] * ua, g2[2] * ub]
                        acc1 = t1 if b == 0 else [x + y for x, y in zip(acc1, t1)]
                for i, acc in enumerate((acc1, acc2)):
                    Yb[i, r0:r0 + RG, ls] = (acc[0] - acc[2]).astype(bf16)
                    Yb[i, PB + r0:PB + r0 + RG, ls] = (acc[0] + acc[1]).astype(bf16)
                return Yb[z + 1, PB + r0:PB + r0 + 16, l0:l0 + 128]

            return [_Gated(functools.partial(task, r0, l0)) for r0 in range(0, PB, RG) for l0 in range(0, D, LG)]

        def job_inv(j, prev=()):
            Yb[z + 2, 0:16, 0:128] = jnp.zeros((16, 128), bf16)
            fiv = after(fi[...], prev)
            srcs = []
            for i in range(2):
                yc = _dot(fiv, Yb[i])
                srcs += _pieces(yc, 2)
                y = yc + ubuf[i * PB:(i + 1) * PB, :].astype(f32) * skt[4:5, :]
                ybuf[rows_at(j * TM + i * PB, PB), :] = y.astype(bf16)
            return srcs

        def tasks_ln(p, res, from_q=False, with_dl=True, mem=False):
            j = rem(p, T)
            s3, s4 = rem(p, 3), rem(p, 4)
            res['t'] = [None] * 16

            def task(k):
                rows = rows_at(j * TM + k * 16, 16)
                x = qb[rows, :].astype(f32) if from_q else xb[rows, :]
                xa = x + _ln(x) * ybuf[rows, :].astype(f32)
                xin = _ln(xa)
                res['t'][k] = _ln(xin).astype(bf16)
                if mem:
                    tbuf[p % 2, k * 16:(k + 1) * 16, :] = res['t'][k]
                xab[s3, k * 16:(k + 1) * 16, :] = xa + xin
                xinb[s4, k * 16:(k + 1) * 16, :] = xin
                if not with_dl:
                    return None
                return res['t'][k][:, 0:128]

            return [functools.partial(task, k) for k in range(16)]

        def tasks_ln2(p):
            j = rem(p, T)
            s4 = rem(p, 4)

            def task(k, gate=None):
                if gate is not None:
                    xinb[z + 4, k * 16:(k + 1) * 16, 0:128] = jnp.concatenate([gate, gate], axis=0)
                zv = _ln(xinb[s4, k * 16:(k + 1) * 16, :]).astype(bf16)
                zbuf[rem(p, 2), k * 16:(k + 1) * 16, :] = zv
                return zv[:, 0:128]

            return [_Gated(functools.partial(task, k)) for k in range(16)]

        def job_w1(p, res, prev=(), dls=()):
            j = rem(p, T)
            tt = tbuf[p % 2] if res is None else jnp.concatenate(res['t'], axis=0)
            pre = _dot(after(tt, prev), need(w1[...], dls, 0.1))
            h = _gelu(pre)
            me = j + 1
            for g, sh in enumerate(SHIFTS):
                ls = slice(g * C4, (g + 1) * C4)
                hg = h[:, ls]
                if sh > 0:
                    hs3[me, sh:TM, ls] = hg[0:TM - sh]
                    hs3[me + 1, 0:sh, ls] = hg[TM - sh:TM]
                else:
                    hs3[me, 0:TM + sh, ls] = hg[-sh:TM]
                    hs3[me - 1, TM + sh:TM, ls] = hg[0:-sh]
            return _pieces(pre)

        def job_w2(p, dls=(), prev=(), lo=0.0):
            j = rem(p, T)
            s3, s4 = rem(p, 3), rem(p, 4)
            hs = _dot(after(hs3[j + 1].astype(bf16), prev), need(w2[...], dls, lo))
            xinb[z + s4 if is_static(s4) else s4] = xinb[s4] + hs
            baseb[rem(p, 2)] = xab[s3] + hs
            return _pieces(hs)

        def m_begin(p):
            rows = rows_at(rem(p, T) * TM, TM)
            return dict(rows=rows, s2=rem(p, 2), z=zbuf[rem(p, 2)])

        def job_m(st, c, t3=(), t4=()):
            zin = after(st['z'], st.pop('prev', st.get('last', ()))) if mchain else st['z']
            pre = _dot(zin, need(w3[:, c * FC:(c + 1) * FC], st.pop('dl', [])))
            hh = _gelu(pre).astype(bf16)
            part = _dot(hh, need(w4[c * FC:(c + 1) * FC, :], _run(t3, _pieces(pre) if gates else None)))
            st['acc'] = (st['acc'] if c else baseb[st['s2']]) + part
            st['dl'] = _run(t4, _pieces(part) if gates else None)
            st['last'] = _pieces(part)

        def m_end(st, to_x, to_o):
            if to_x:
                xb[st['rows'], :] = st['acc']
            if to_o:
                obuf[st['rows'], :] = st['acc'].astype(bf16)

        def m_jobs(st, tasks, c0=0, c1=None):
            c1 = NFC if c1 is None else c1
            n = 2 * (c1 - c0) - 1
            parts = _split(tasks, n) + [[]]
            for c in range(c0, c1):
                job_m(st, c, parts[2 * (c - c0)], parts[2 * (c - c0) + 1])

        def mac_under_w1(c, p, res, prev):
            dm = _run(tasks_mac(c))
            nd = min(len(dm), int(a_macrate * 4096 / (26 * (4 * c + 3))))
            dm = dm[:nd]
            if mac_nd is not None:
                step = max(1, nd // mac_nd) if mac_nd else 10 ** 6
                dm = dm[step - 1::step]
            return job_w1(p, res, prev, dm)

        def step_b(t):
            res = {}
            if t == 0:
                prev = job_h(0, g_fence=True)
                release(prev, k=True)
                _run(tasks_kv(0, False))
                prev = job_u(0, prev)
                _run(tasks_mac(0))
                prev = job_h(1, prev)
                job_inv(0, prev)
            elif t == 1:
                prev = job_h(2)
                release(prev, k=True, q=True)
                _run(tasks_kv(1, False))
                _run(tasks_ln(0, res, from_q=True, with_dl=False, mem=True))
                prev = job_u(1, prev)
                _run(tasks_mac(1))
                job_inv(1, prev)
            else:
                prev = job_w1(0, None) if t == 2 else job_w2(0)
                release(prev, k=True)
                _run(tasks_kv(t, t == 3))
                release(prev, q=True)
                _run(tasks_ln(t - 1, res, from_q=True, with_dl=False))
                if t == 3:
                    _run(tasks_ln2(0))
                prev = job_u(t, prev)
                dm = _run(tasks_mac(t))
                prev = job_h(t + 1, prev)
                nd = min(len(dm), int(a_macrate * 5120 / (26 * (4 * t + 3))))
                step = max(1, nd // mac_nd) if mac_nd else 10 ** 6
                prev = job_w1(t - 1, res, prev, dm[:nd][step - 1::step])
                job_inv(t, prev)

        def body_mc(t, midwait=None):
            res = {}
            st = m_begin(t - 4)
            cu = 1 if midwait is None else 3
            prev = job_w2(t - 3)
            release(prev, k=True, q=True)
            _run(tasks_kv(t, True))
            ln2 = tasks_ln2(t - 3)
            for c in range(cu):
                job_m(st, c, ln2 if c == cu - 1 else [])
            if midwait is not None:
                midwait()
            if mac_gate:
                job_u(t, fence=False)
                nj = 2 * (NFC - cu) - 1
                nodl = lambda f: _Gated(lambda gate=None: (f(gate), None)[1])
                tm = tasks_mac(t, mac_gate)
                if not mac_gdl:
                    tm = [nodl(f) for f in tm]
                pm = _split(tm, nj - mac_slack) + [[]] * mac_slack
                pn = _split(tasks_ln(t - 1, res), nj)
                tasks = [_interleave(a, b) for a, b in zip(pm, pn)] + [[]]
                c_ln = cu
            else:
                job_u(t)
                _run(tasks_mac(t))
                c_ln = max(cu, ln_from)
                tasks = _split(tasks_ln(t - 1, res), 2 * (NFC - c_ln) - 1) + [[]]
            for c in range(cu, NFC):
                if c >= c_ln:
                    job_m(st, c, tasks[2 * (c - c_ln)], tasks[2 * (c - c_ln) + 1])
                else:
                    job_m(st, c)
                if c == h_after and t + 1 < T:
                    job_h(t + 1)
            m_end(st, True, False)
            job_inv(t)
            job_w1(t - 1, res)

        def body_mpr(t, carry):
            res = {}
            st = m_begin(t - 4)
            job_w2(t - 3)
            m_jobs(st, tasks_ln2(t - 3) + tasks_ln(t - 1, res))
            m_end(st, True, True)
            job_w1(t - 1, res)

            @pl.when(t - 4 >= T)
            def _():
                out_copy(t - 4 - T).start()
            return carry

        def body_mr(t, carry):
            st = m_begin(t - 4)
            job_w2(t - 3)
            m_jobs(st, tasks_ln2(t - 3))
            m_end(st, False, True)
            out_copy(t - 4 - T).start()
            return carry

        def body_m(t):
            st = m_begin(t - 4)
            m_jobs(st, [])
            m_end(st, False, True)
            out_copy(t - 4 - T).start()

        if only is not None:
            @pl.when(z == 0)
            def _():
                if isinstance(only, int):
                    step_b(only) if only < 4 else body_mc(only)
                else:
                    dict(mpr=body_mpr, mr=body_mr)[only](z + 4 + T, 0)
            zz = pl.ds(z16, 16)
            obuf[0:16, :] = (ybuf[zz, :] + zbuf[z, zz, :] + Yb[z, zz, :] + tbuf[z, zz, :]
                             + (hs3[z, zz, :] + U[z, zz, :] + G[z, zz, :] + hprev[zz, :]
                                + xab[z, zz, :] + xinb[z, zz, :] + xb[zz, :] + baseb[z, zz, :]).astype(bf16))
            out_copy(0).start()
            out_copy(0).wait()
            return

        scope = jax.named_scope if scopes else (lambda name: contextlib.nullcontext())

        def tile(j):
            return [in_copy(1, j), in_copy(2, j)] + ([in_copy(0, j + 1)] if j + 1 < T else [])

        def qs(*js):
            return [in_copy(3, j) for j in js]

        def chunks(lo, hi):
            return [cp for c in range(lo, hi) for cp in w34_copies(c)]

        starts = {
            0: lambda: ([w_copy(2), w_copy(3), in_copy(0, 0)] + tile(0) + tile(1) + qs(0) + [w_copy(0)] + qs(1) + tile(2)
                        + [w_copy(1)] + tile(3) + qs(2, 3)),
            1: lambda: chunks(0, 3) + tile(4) + qs(4),
            2: lambda: chunks(3, NFC) + tile(5) + qs(5),
            3: lambda: tile(6) + qs(6),
            4: lambda: tile(7) + qs(7),
        }
        waits = {
            0: lambda: [in_copy(0, 0)] + tile(0),
            1: lambda: tile(1) + qs(0),
            2: lambda: [w_copy(0)] + qs(1) + tile(2),
            3: lambda: [w_copy(1)] + tile(3) + qs(2, 3),
            4: lambda: chunks(0, 3) + tile(4) + qs(4),
            5: lambda: tile(5) + qs(5),
            6: lambda: tile(6) + qs(6),
            7: lambda: tile(7) + qs(7),
        }

        def midwait():
            for cp in chunks(3, NFC):
                cp.wait()

        for cp in starts[0]():
            cp.start()
        with scope("const"):
            pl.when(z == 0)(constants)
        w_copy(2).wait()
        w_copy(3).wait()
        skt[0:4, :] = sk_ref[...].astype(f32)
        skt[4:8, :] = jnp.broadcast_to(dv_ref[...].astype(f32).reshape(1, D), (4, D))
        for t in range(T):
            if t > 0 and t in starts:
                for cp in starts[t]():
                    cp.start()
            with scope(f"wait{t}"):
                for cp in waits[t]():
                    cp.wait()
            with scope(f"step{t}"):
                @pl.when(z == 0)
                def _(t=t):
                    if t < 4:
                        step_b(t)
                    else:
                        body_mc(t, midwait if t == 4 else None)
        with scope("loopMPR"):
            lax.fori_loop(T, 2 * T + 1, body_mpr, 0)
        with scope("loopMR"):
            lax.fori_loop(2 * T + 1, 2 * T + 3, body_mr, 0)
        with scope("lastM"):
            body_m(2 * T + 3)
        with scope("waitO"):
            for j in range(T):
                out_copy(j).wait()

    @jax.jit
    def fn(A_q, A_k, A_v, A_shift_k, A_ssm_k, A_ssm_D, B_x, B_w1, B_w2, B_w3, B_w4):
        any_spec = pl.BlockSpec(memory_space=pl.ANY)
        scratch = [
            pltpu.VMEM((S + 64, D), bf16),
            pltpu.VMEM((NIN + 1, TM, D), bf16),
            pltpu.VMEM((NIN, TM, D), bf16),
            pltpu.VMEM((NIN, D, TM), bf16),
            pltpu.VMEM((D, D), bf16),
            pltpu.VMEM((D, D), bf16),
            pltpu.VMEM((D, F), bf16),
            pltpu.VMEM((F, D), bf16),
            pltpu.VMEM((4, D), bf16),
            pltpu.VMEM((D,), bf16),
            pltpu.VMEM((2 * PB, PB), bf16),
            pltpu.VMEM((PB, 2 * PB), bf16),
            pltpu.VMEM((8, D), f32),
            pltpu.VMEM((8, D), f32),
            pltpu.VMEM((2 * PB, D), f32),
            pltpu.VMEM((NB + 1, 2 * PB, D), f32),
            pltpu.VMEM((NB + 1, 3 * PB, D), f32),
            pltpu.VMEM((3, 2 * PB, D), bf16),
            pltpu.VMEM((S + 32, D), f32),
            pltpu.VMEM((S, D), bf16),
            pltpu.VMEM((T + 2, TM, D), f32),
            pltpu.VMEM((3, TM, D), f32),
            pltpu.VMEM((5, TM, D), f32),
            pltpu.VMEM((2, TM, D), bf16),
            pltpu.VMEM((S, D), bf16),
            pltpu.VMEM((TM + 16, D), bf16),
            pltpu.VMEM((2, TM, D), bf16),
            pltpu.VMEM((4, 2 * (TM + 8), 128), f32),
            pltpu.VMEM((2, TM, D), f32),
            pltpu.SemaphoreType.DMA((5 * T + 4 + 2 * NFC,)),
        ]
        return pl.pallas_call(
            kernel,
            in_specs=[any_spec] * 10,
            out_specs=any_spec,
            out_shape=jax.ShapeDtypeStruct((1, S, D), bf16),
            scratch_shapes=scratch,
            compiler_params=pltpu.CompilerParams(vmem_limit_bytes=124 * 1024 * 1024),
        )(A_q, A_k, A_v, A_shift_k.T, A_ssm_k, A_ssm_D, B_w1, B_w2, B_w3, B_w4)

    return fn


_impl = make()


@jax.jit
def pallas_interleave_layers__ssm_conv_h3__mixer_s_mlp__prompt_kernel(
        A_q, A_k, A_v, A_shift_k, A_ssm_k, A_ssm_D, B_x, B_w1, B_w2, B_w3, B_w4):
    return _impl(A_q, A_k, A_v, A_shift_k, A_ssm_k, A_ssm_D, B_x, B_w1, B_w2, B_w3, B_w4)
```

```python
import contextlib
import functools
import math

import jax
import jax.numpy as jnp
from jax import lax
import jax.experimental.pallas as pl
import jax.experimental.pallas.tpu as pltpu

S = 2048
D = 1024
F = 3584
TM = 256
T = S // TM
PB = 128
NB = S // PB
FC = 512
NFC = F // FC
EPS = 1e-5
SHIFTS = (1, -1, 2, -2)
NIN = 4
NLAST = 4
f32 = jnp.float32
bf16 = jnp.bfloat16


def _ln(x):
    m = jnp.mean(x, axis=-1, keepdims=True)
    xc = x - m
    v = jnp.mean(xc * xc, axis=-1, keepdims=True)
    return xc * lax.rsqrt(v + EPS)


def _ln_centered(x):
    n = x.shape[-1]
    m = jnp.sum(x, axis=-1, keepdims=True) * (1.0 / n)
    ms = jnp.sum(x * x, axis=-1, keepdims=True) * (1.0 / n)
    v = jnp.maximum(ms - m * m, 0.0)
    return (x - m) * lax.rsqrt(v + EPS)


def _gelu(x):
    c = math.sqrt(2.0 / math.pi)
    inner = x * (c + (c * 0.044715) * (x * x))
    hx = 0.5 * x
    return hx + hx * jnp.tanh(inner)


def _dot(a, b):
    return jnp.dot(a, b, preferred_element_type=f32)


def _dot_nt(a, b):
    return lax.dot_general(a, b, (((1,), (1,)), ((), ())), preferred_element_type=f32)


def _pieces(val, ngroup=1):
    rows, cols = val.shape
    return [functools.partial(lambda r, n: val[r * 8:(r + 1) * 8, n * 128:(n + 1) * 128], r, n)
            for n in range(0, cols // 128, ngroup) for r in range(rows // 8)]


class _Gated:
    def __init__(self, fn):
        self.fn = fn

    def __call__(self, gate=None):
        return self.fn(gate=gate)


def _run(tasks, srcs=None):
    out = []
    for i, task in enumerate(tasks):
        if srcs and isinstance(task, _Gated):
            out.append(task(srcs[(i * len(srcs)) // len(tasks)]()))
        else:
            out.append(task())
    return out


def _interleave(*lists):
    items = [((i + 0.5) / len(l), li, x) for li, l in enumerate(lists) for i, x in enumerate(l)]
    items.sort(key=lambda e: (e[0], e[1]))
    return [e[2] for e in items]


def _split(tasks, n):
    return [tasks[(i * len(tasks)) // n:((i + 1) * len(tasks)) // n] for i in range(n)]


def _twice(d):
    return jnp.concatenate([d, d], axis=0).astype(bf16)


def make(only=None, only_part=None, scopes=False,
         c_inv=2, c_kv=2, c_u=6, h_split=(3, 5), mc_rel=0.1, b1_ln=4, b_ln=0.8):

    def kernel(q_hbm, k_hbm, v_hbm, sk_hbm, hk_hbm, dv_hbm, w1_hbm, w2_hbm, w3_hbm, w4_hbm,
               o_hbm,
               qb, kb, vb, hkb, w1, w2, w3, w4, sk_ref, dv_ref, ff, fi, skt, hprev, U, G, Yb,
               xb, ybuf, hs3, xab, xinb, zbuf, obuf, ubuf, tbuf, kst, baseb, accb,
               sems):
        def is_static(j):
            return isinstance(j, int)

        def rows_at(r0, n):
            return pl.ds(r0 if is_static(r0) else pl.multiple_of(r0, n), n)

        def rem(j, n):
            return j % n if is_static(j) else lax.rem(j, n)

        def hk(j):
            return [pltpu.make_async_copy(hk_hbm.at[:, pl.ds(j * TM, TM)], hkb.at[j % NIN], sems.at[j])]

        def kv_in(j):
            rows = pl.ds(j * TM, TM)
            return [pltpu.make_async_copy(k_hbm.at[0, rows, :], kb.at[j % NIN], sems.at[T + j]),
                    pltpu.make_async_copy(v_hbm.at[0, rows, :], vb.at[j % NIN], sems.at[2 * T + j])]

        def tile(j):
            return hk(j) + kv_in(j)

        def qs(j):
            rows = pl.ds(j * TM, TM)
            return [pltpu.make_async_copy(q_hbm.at[0, rows, :], qb.at[rows, :], sems.at[3 * T + j])]

        def whole(i):
            src, dst = [(w1_hbm, w1), (w2_hbm, w2), (sk_hbm, sk_ref), (dv_hbm, dv_ref)][i]
            return [pltpu.make_async_copy(src, dst, sems.at[4 * T + i])]

        def chunks(lo, hi):
            out = []
            for c in range(lo, hi):
                cs = pl.ds(c * FC, FC)
                out += [pltpu.make_async_copy(w3_hbm.at[:, cs], w3.at[:, cs], sems.at[4 * T + 4 + 2 * c]),
                        pltpu.make_async_copy(w4_hbm.at[cs, :], w4.at[cs, :], sems.at[4 * T + 5 + 2 * c])]
            return out

        def out_copy(j):
            rows = rows_at(j * TM, TM)
            return pltpu.make_async_copy(obuf.at[rows, :], o_hbm.at[0, rows, :], sems.at[4 * T + 4 + 2 * NFC + j])

        def last_copy(n):
            rows = pl.ds((T - 1) * TM, TM)
            cs = pl.ds(n * (D // NLAST), D // NLAST)
            return pltpu.make_async_copy(obuf.at[rows, cs], o_hbm.at[0, rows, cs], sems.at[5 * T + 3 + 2 * NFC + n])

        def start_all(cps):
            for cp in cps:
                cp.start()

        def wait_all(cps):
            for cp in cps:
                cp.wait()

        z = jnp.min(lax.broadcasted_iota(jnp.int32, (8, 128), 1))
        never = z > 0
        z16 = pl.multiple_of(z, 16)

        def need(w, dls):
            dls = [d for d in dls if d is not None]
            if not dls:
                return w
            nt = w.shape[1] // 128
            cols = [w[:, n * 128:(n + 1) * 128] for n in range(nt)]
            npass = w.shape[0] // 512
            used = {}
            for i, d in enumerate(dls):
                slot = ((i + 1) * nt * npass - 1) // len(dls)
                used[slot] = used.get(slot, -1) + 1
                n, r0 = slot // npass, (slot % npass) * 512 + 16 * used[slot]
                parts = [cols[n][:r0]] if r0 else []
                parts += [jnp.where(never, d, cols[n][r0:r0 + 16]), cols[n][r0 + 16:]]
                cols[n] = jnp.concatenate(parts, axis=0)
            return jnp.concatenate(cols, axis=1)

        def after(x, srcs):
            if not srcs:
                return x
            head = jnp.where(never, _twice(srcs[max(0, len(srcs) - 33)]()), x[:16, :128])
            if x.shape[1] > 128:
                head = jnp.concatenate([head, x[:16, 128:]], axis=1)
            return jnp.concatenate([head, x[16:]], axis=0)

        def release_k(srcs):
            for i in range(32):
                kb[z + NIN, 16 * (i // 8):16 * (i // 8) + 16, (i % 8) * 128:(i % 8 + 1) * 128] = _twice(srcs[i]())

        def release_u(srcs):
            for i in range(32):
                U[z + NB, 8 * i:8 * i + 8, 0:128] = srcs[i]()

        def release_g(srcs):
            for i in range(32):
                G[z + NB - 1, 8 * i:8 * i + 8, 0:128] = srcs[i]()

        def constants():
            r = lax.broadcasted_iota(jnp.int32, (2 * PB, PB), 0)
            t = lax.broadcasted_iota(jnp.int32, (2 * PB, PB), 1)
            slot = ((r >> 4) << 3) + (r & 7)
            freq = jnp.where(slot < 64, 2 * slot, 2 * slot - 127)
            phase = ((2 * freq + 1) * t + jnp.where((r & 8) != 0, 128, 0)) & 511
            fw = jnp.cos(phase.astype(f32) * (2.0 * math.pi / 512.0))
            ff[...] = fw.astype(bf16)
            fi[...] = (fw.T * (1.0 / PB)).astype(bf16)
            kst[:, 0:16, :] = jnp.zeros((4, 16, 128), f32)
            hs3[1, 0:8, :] = jnp.zeros((8, D), f32)
            hs3[T, TM - 8:TM, :] = jnp.zeros((8, D), f32)

        def job_h(j, prev=(), quarters=range(4)):
            ffv = after(ff[...], prev)
            srcs = []
            LQ = D // 4
            for qd in quarters:
                ls = slice(qd * LQ, (qd + 1) * LQ)
                hh = _dot_nt(ffv, jnp.concatenate([hkb[j % NIN, ls, 0:PB], hkb[j % NIN, ls, PB:2 * PB]], axis=0))
                srcs += _pieces(hh, 4)
                for g in range(PB // 8):
                    re, im = hh[16 * g:16 * g + 8], hh[16 * g + 8:16 * g + 16]
                    blocks = [(re[:, :LQ], im[:, :LQ]), (re[:, LQ:], im[:, LQ:])]
                    for i in range(2):
                        gr, gi = blocks[i]
                        if 2 * j + i > 0:
                            pr, pi_ = blocks[0] if i else (hprev[16 * g:16 * g + 8, ls],
                                                           hprev[16 * g + 8:16 * g + 16, ls])
                            gr, gi = (gr - pi_, gi + pr) if g < 8 else (gr + pi_, gi - pr)
                        G[2 * j + i, 8 * g:8 * g + 8, ls] = gr
                        G[2 * j + i, PB + 8 * g:PB + 8 * g + 8, ls] = gi - gr
                        G[2 * j + i, 2 * PB + 8 * g:2 * PB + 8 * g + 8, ls] = gr + gi
                    if j < T - 1:
                        hprev[16 * g:16 * g + 16, ls] = hh[16 * g:16 * g + 16, LQ:]
            return srcs

        def tasks_kv(j):
            sl = j % NIN

            def task(i, lt, gate=None):
                ls = slice(lt * 128, (lt + 1) * 128)
                rs = slice(i * PB, (i + 1) * PB)
                if gate is not None:
                    kb[z + NIN, pl.ds(z16, 16), ls] = _twice(gate)
                kf = kb[sl, rs, ls].astype(f32)
                pair, par = lt // 2, lt % 2
                kst[pair, pl.ds(2 * (8 + i * PB) + par, PB, stride=2), :] = kf
                ks = kf * skt[0:1, ls]
                for tt in range(1, 4):
                    ks = ks + kst[pair, pl.ds(2 * (8 - tt + i * PB) + par, PB, stride=2), :] * skt[tt:tt + 1, ls]
                if i == 1:
                    kst[pair, pl.ds(par, 8, stride=2), :] = kf[PB - 8:]
                ubuf[j % 2, rs, ls] = (ks * vb[sl, rs, ls].astype(f32)).astype(bf16)
                return ubuf[j % 2, pl.ds(z16 + i * PB, 16), ls]

            return [_Gated(functools.partial(task, i, lt)) for i in range(2) for lt in range(8)]

        def job_u(j, prev=()):
            ubuf[j % 2, pl.ds(z16 + TM, 16), 0:128] = jnp.zeros((16, 128), bf16)
            ffv = after(ff[...], prev)
            srcs = []
            for i in range(2):
                uu = _dot(ffv, ubuf[j % 2, i * PB:(i + 1) * PB, :])
                srcs += _pieces(uu, 4)
                U[2 * j + i] = uu
            return srcs

        def run_mac(j):
            for r0 in range(0, PB, 8):
                for l0 in range(0, D, 256):
                    ls = slice(l0, l0 + 256)
                    gld = lambda c: [G[c, p * PB + r0:p * PB + r0 + 8, ls] for p in range(3)]
                    acc = [None, None]
                    g = gld(2 * j + 1)
                    for b in range(2 * j + 2):
                        ua, ub = U[b, 2 * r0:2 * r0 + 8, ls], U[b, 2 * r0 + 8:2 * r0 + 16, ls]
                        us = ua + ub
                        for i in (1, 0):
                            if 2 * j + i - b >= 0:
                                if i == 0:
                                    g = gld(2 * j - b)
                                term = [g[0] * us, g[1] * ua, g[2] * ub]
                                acc[i] = term if b == 0 else [x + y for x, y in zip(acc[i], term)]
                    for i in range(2):
                        Yb[i, 2 * r0:2 * r0 + 16, ls] = jnp.concatenate(
                            [acc[i][0] - acc[i][2], acc[i][0] + acc[i][1]], axis=0).astype(bf16)

        def job_inv(j, prev=()):
            Yb[z + 2, 0:16, 0:128] = jnp.zeros((16, 128), bf16)
            fiv = after(fi[...], prev)
            srcs = []
            for i in range(2):
                yc = _dot(fiv, Yb[i])
                srcs += _pieces(yc, 2)
                y = yc + ubuf[j % 2, i * PB:(i + 1) * PB, :].astype(f32) * skt[4:5, :]
                ybuf[j * TM + i * PB:j * TM + (i + 1) * PB, :] = y.astype(bf16)
            return srcs

        def tasks_ln(p, res, gated=False, mem=False):
            j = rem(p, T)
            s3, s4 = rem(p, 3), rem(p, 4)
            res['t'] = [None] * 16

            def task(k, gate=None):
                rows = rows_at(j * TM + k * 16, 16)
                if gate is not None:
                    qb[pl.ds(z16 + S, 16), 0:128] = _twice(gate)
                x = qb[rows, :].astype(f32) if is_static(p) else xb[rows, :]
                xa = x + _ln(x) * ybuf[rows, :].astype(f32)
                xin = _ln(xa)
                res['t'][k] = _ln_centered(xin).astype(bf16)
                if mem:
                    tbuf[p % 2, k * 16:(k + 1) * 16, :] = res['t'][k]
                xab[s3, k * 16:(k + 1) * 16, :] = xa + xin
                xinb[s4, k * 16:(k + 1) * 16, :] = xin
                return res['t'][k][:, 0:128]

            wrap = _Gated if gated else (lambda f: f)
            return [wrap(functools.partial(task, k)) for k in range(16)]

        def tasks_ln2(p):
            def task(k, gate=None):
                if gate is not None:
                    xinb[z + 4, k * 16:(k + 1) * 16, 0:128] = jnp.concatenate([gate, gate], axis=0)
                zv = _ln(xinb[rem(p, 4), k * 16:(k + 1) * 16, :]).astype(bf16)
                zbuf[rem(p, 2), k * 16:(k + 1) * 16, :] = zv
                return zv[:, 0:128]

            return [_Gated(functools.partial(task, k)) for k in range(16)]

        def job_w1(p, res, prev=()):
            tt = tbuf[p % 2] if res is None else jnp.concatenate(res['t'], axis=0)
            pre = _dot(after(tt, prev), w1[...])
            h = _gelu(pre)
            me = rem(p, T) + 1
            for g, sh in enumerate(SHIFTS):
                ls = slice(g * (D // 4), (g + 1) * (D // 4))
                hg = h[:, ls]
                if sh > 0:
                    hs3[me, sh:TM, ls] = hg[0:TM - sh]
                    hs3[me + 1, 0:sh, ls] = hg[TM - sh:TM]
                else:
                    hs3[me, 0:TM + sh, ls] = hg[-sh:TM]
                    hs3[me - 1, TM + sh:TM, ls] = hg[0:-sh]
            return _pieces(pre)

        def job_w2(p):
            s4 = rem(p, 4)
            hs = _dot(hs3[rem(p, T) + 1].astype(bf16), w2[...])
            xinb[z + s4 if is_static(s4) else s4] = xinb[s4] + hs
            baseb[rem(p, 2)] = xab[rem(p, 3)] + hs
            return _pieces(hs)

        def m_begin(p):
            return dict(rows=rows_at(rem(p, T) * TM, TM), s2=rem(p, 2), z=zbuf[rem(p, 2)])

        def job_m(st, c, t3=(), t4=()):
            pre = _dot(st['z'], need(w3[:, c * FC:(c + 1) * FC], st.pop('dl', [])))
            hh = _gelu(pre).astype(bf16)
            part = _dot(hh, need(w4[c * FC:(c + 1) * FC, :], _run(t3, _pieces(pre))))
            st['acc'] = (st['acc'] if c else baseb[st['s2']]) + part
            st['dl'] = _run(t4, _pieces(part))

        def m_jobs(st, tasks):
            parts = _split(tasks, 2 * NFC - 1) + [[]]
            for c in range(NFC):
                job_m(st, c, parts[2 * c], parts[2 * c + 1])

        def step_b0(mid):
            _run(tasks_kv(0))
            prev = job_u(0)
            release_u(prev[-32:])
            run_mac(0)
            job_inv(0, prev)
            mid()
            job_h(1)

        def step_b1():
            res = {}
            _run(tasks_kv(1))
            ln = tasks_ln(0, res, gated=True, mem=True)
            _run(ln[:b1_ln])
            prev = job_u(1)
            release_u(prev[-32:])
            _run(ln[b1_ln:], prev)
            run_mac(1)
            job_inv(1, prev)

        def step_b2(mid):
            prev = job_w1(0, None)
            release_k(prev)
            _run(tasks_kv(2))
            _run(tasks_ln(1, {}, gated=True, mem=True), prev[:int(len(prev) * b_ln)])
            job_u(2, prev)
            mid()
            ph = job_h(2)
            release_g(ph[-32:])
            prev = job_w1(1, None, ph)
            release_u(ph[-32:])
            run_mac(2)
            job_inv(2, prev)

        def step_b3():
            res = {}
            prev = job_w2(0)
            release_k(prev)
            _run(tasks_kv(3))
            _run(tasks_ln(2, res, gated=True), prev[:int(len(prev) * b_ln)])
            prev = job_u(3, prev)
            prev = job_h(3, prev)
            prev = job_w1(2, res, prev)
            _run(tasks_ln2(0), prev[:len(prev) * 3 // 4])

        def step_mc_a(t):
            st = m_begin(t - 4)
            prev = job_w2(t - 3)
            release_u(prev[int(len(prev) * mc_rel):])
            run_mac(t - 1)
            for c in range(c_inv + 1):
                job_m(st, c, tasks_ln2(t - 3) if c == c_inv else ())
            accb[...] = st['acc']
            job_inv(t - 1)

        def step_mc_b(t, mid=None):
            res = {}
            st = m_begin(t - 4)
            st['acc'] = accb[...]
            ckv = 4 if mid else c_kv
            ln = _split(tasks_ln(t - 1, res), 2 * (NFC - c_inv - 1) - 1) + [[]]
            kv = _split(tasks_kv(t) if t < T else [], 2 * (c_u - ckv) - 1) + [[]]
            for c in range(c_inv + 1, NFC):
                if mid and c == 5:
                    mid()
                t3, t4 = ln[2 * (c - c_inv - 1)], ln[2 * (c - c_inv - 1) + 1]
                if ckv < c <= c_u:
                    t3 = _interleave(t3, kv[2 * (c - ckv - 1)])
                    t4 = _interleave(t4, kv[2 * (c - ckv - 1) + 1])
                job_m(st, c, t3, t4)
                if t < T:
                    if c == c_u:
                        job_u(t)
                    if mid:
                        if c == NFC - 1:
                            job_h(t)
                    elif c in h_split:
                        job_h(t, quarters=(2 * h_split.index(c), 2 * h_split.index(c) + 1))
            xb[st['rows'], :] = st['acc']
            job_w1(t - 1, res)

        def body_mpr(t, carry):
            res = {}
            st = m_begin(t - 4)
            job_w2(t - 3)
            m_jobs(st, tasks_ln2(t - 3) + tasks_ln(t - 1, res))
            xb[st['rows'], :] = st['acc']
            obuf[st['rows'], :] = st['acc'].astype(bf16)
            job_w1(t - 1, res)

            @pl.when(t - 4 >= T)
            def _():
                out_copy(t - 4 - T).start()
            return carry

        def body_mr(t, carry):
            st = m_begin(t - 4)
            job_w2(t - 3)
            m_jobs(st, tasks_ln2(t - 3))
            obuf[st['rows'], :] = st['acc'].astype(bf16)
            out_copy(t - 4 - T).start()
            return carry

        def step_last():
            st = m_begin(2 * T - 1)
            m_jobs(st, [])
            for n in range(NLAST):
                cs = slice(n * (D // NLAST), (n + 1) * (D // NLAST))
                obuf[st['rows'], cs] = st['acc'][:, cs].astype(bf16)
                last_copy(n).start()

        scope = jax.named_scope if scopes else (lambda name: contextlib.nullcontext())
        nreg = [0]

        def region(name, fn, *args):
            nreg[0] += 1
            with scope(name):
                pl.when(z <= nreg[0])(lambda: (fn(*args), None)[1])

        def waits(name, cps):
            with scope("w" + name):
                wait_all(cps)

        start_all(hk(0) + whole(2) + whole(3) + kv_in(0) + hk(1) + kv_in(1) + qs(0) + whole(0) + qs(1)
                  + kv_in(2) + hk(2) + whole(1) + hk(3) + qs(2) + kv_in(3))
        region("const", constants)
        waits("h0", hk(0))
        region("h0", job_h, 0)
        wait_all(whole(2) + whole(3))
        skt[0:4, :] = sk_ref[...].astype(f32)
        skt[4:8, :] = jnp.broadcast_to(dv_ref[...].astype(f32).reshape(1, D), (4, D))
        waits("b0", kv_in(0))
        region("b0", step_b0, lambda: wait_all(hk(1)))
        start_all(chunks(0, 4) + qs(3) + chunks(4, NFC) + tile(4))
        waits("b1", kv_in(1) + qs(0))
        region("b1", step_b1)
        start_all(qs(4) + tile(5))
        waits("b2", whole(0) + qs(1) + kv_in(2))
        region("b2", step_b2, lambda: wait_all(hk(2)))
        start_all(qs(5) + tile(6))
        waits("b3", whole(1) + hk(3) + qs(2) + kv_in(3))
        region("b3", step_b3)
        start_all(qs(6) + tile(7) + qs(7))
        waits("4a", chunks(0, 3))
        region("mc4a", step_mc_a, 4)
        waits("4b", chunks(3, 4) + qs(3) + chunks(4, 5))
        region("mc4b", step_mc_b, 4, lambda: wait_all(chunks(5, NFC) + tile(4)))
        for t in range(5, T + 1):
            region(f"mc{t}a", step_mc_a, t)
            waits(f"{t}b", qs(t - 1) + (tile(t) if t < T else []))
            region(f"mc{t}b", step_mc_b, t)
        with scope("loopMPR"):
            lax.fori_loop(T + 1, 2 * T + 1, body_mpr, 0)
        with scope("loopMR"):
            lax.fori_loop(2 * T + 1, 2 * T + 3, body_mr, 0)
        with scope("last"):
            step_last()
        with scope("waitO"):
            wait_all([out_copy(j) for j in range(T - 1)] + [last_copy(n) for n in range(NLAST)])

    @jax.jit
    def fn(A_q, A_k, A_v, A_shift_k, A_ssm_k, A_ssm_D, B_x, B_w1, B_w2, B_w3, B_w4):
        scratch = [
            pltpu.VMEM((S + 16, D), bf16),
            pltpu.VMEM((NIN + 1, TM, D), bf16),
            pltpu.VMEM((NIN, TM, D), bf16),
            pltpu.VMEM((NIN, D, TM), bf16),
            pltpu.VMEM((D, D), bf16),
            pltpu.VMEM((D, D), bf16),
            pltpu.VMEM((D, F), bf16),
            pltpu.VMEM((F, D), bf16),
            pltpu.VMEM((4, D), bf16),
            pltpu.VMEM((D,), bf16),
            pltpu.VMEM((2 * PB, PB), bf16),
            pltpu.VMEM((PB, 2 * PB), bf16),
            pltpu.VMEM((8, D), f32),
            pltpu.VMEM((2 * PB, D), f32),
            pltpu.VMEM((NB + 1, 2 * PB, D), f32),
            pltpu.VMEM((NB, 3 * PB, D), f32),
            pltpu.VMEM((3, 2 * PB, D), bf16),
            pltpu.VMEM((S, D), f32),
            pltpu.VMEM((S, D), bf16),
            pltpu.VMEM((T + 2, TM, D), f32),
            pltpu.VMEM((3, TM, D), f32),
            pltpu.VMEM((5, TM, D), f32),
            pltpu.VMEM((2, TM, D), bf16),
            pltpu.VMEM((S, D), bf16),
            pltpu.VMEM((2, TM + 16, D), bf16),
            pltpu.VMEM((2, TM, D), bf16),
            pltpu.VMEM((4, 2 * (TM + 16), 128), f32),
            pltpu.VMEM((2, TM, D), f32),
            pltpu.VMEM((TM, D), f32),
            pltpu.SemaphoreType.DMA((5 * T + 3 + 2 * NFC + NLAST,)),
        ]
        return pl.pallas_call(
            kernel,
            in_specs=[pl.BlockSpec(memory_space=pl.ANY)] * 10,
            out_specs=pl.BlockSpec(memory_space=pl.ANY),
            out_shape=jax.ShapeDtypeStruct((1, S, D), bf16),
            scratch_shapes=scratch,
            compiler_params=pltpu.CompilerParams(vmem_limit_bytes=124 * 1024 * 1024),
        )(A_q, A_k, A_v, A_shift_k.T, A_ssm_k, A_ssm_D, B_w1, B_w2, B_w3, B_w4)

    return fn


_impl = make()


@jax.jit
def pallas_interleave_layers__ssm_conv_h3__mixer_s_mlp__prompt_kernel(
        A_q, A_k, A_v, A_shift_k, A_ssm_k, A_ssm_D, B_x, B_w1, B_w2, B_w3, B_w4):
    return _impl(A_q, A_k, A_v, A_shift_k, A_ssm_k, A_ssm_D, B_x, B_w1, B_w2, B_w3, B_w4)
```

```python
import contextlib
import functools
import math

import jax
import jax.numpy as jnp
from jax import lax
import jax.experimental.pallas as pl
import jax.experimental.pallas.tpu as pltpu

S = 2048
D = 1024
F = 3584
TM = 256
T = S // TM
PB = 128
NB = S // PB
FC = 512
NFC = F // FC
EPS = 1e-5
SHIFTS = (1, -1, 2, -2)
NIN = 4
NLAST = 4
f32 = jnp.float32
bf16 = jnp.bfloat16


def _ln(x):
    m = jnp.mean(x, axis=-1, keepdims=True)
    xc = x - m
    v = jnp.mean(xc * xc, axis=-1, keepdims=True)
    return xc * lax.rsqrt(v + EPS)


def _ln_centered(x):
    n = x.shape[-1]
    m = jnp.sum(x, axis=-1, keepdims=True) * (1.0 / n)
    ms = jnp.sum(x * x, axis=-1, keepdims=True) * (1.0 / n)
    v = jnp.maximum(ms - m * m, 0.0)
    return (x - m) * lax.rsqrt(v + EPS)


def _gelu(x):
    c = math.sqrt(2.0 / math.pi)
    inner = x * (c + (c * 0.044715) * (x * x))
    hx = 0.5 * x
    return hx + hx * jnp.tanh(inner)


def _dot(a, b):
    return jnp.dot(a, b, preferred_element_type=f32)


def _dot_nt(a, b):
    return lax.dot_general(a, b, (((1,), (1,)), ((), ())), preferred_element_type=f32)


def _pieces(val, ngroup=1):
    rows, cols = val.shape
    return [functools.partial(lambda r, n: val[r * 8:(r + 1) * 8, n * 128:(n + 1) * 128], r, n)
            for n in range(0, cols // 128, ngroup) for r in range(rows // 8)]


class _Gated:
    def __init__(self, fn):
        self.fn = fn

    def __call__(self, gate=None):
        return self.fn(gate=gate)


def _run(tasks, srcs=None):
    out = []
    for i, task in enumerate(tasks):
        if srcs and isinstance(task, _Gated):
            out.append(task(srcs[(i * len(srcs)) // len(tasks)]()))
        else:
            out.append(task())
    return out


def _interleave(*lists):
    items = [((i + 0.5) / len(l), li, x) for li, l in enumerate(lists) for i, x in enumerate(l)]
    items.sort(key=lambda e: (e[0], e[1]))
    return [e[2] for e in items]


def _split(tasks, n):
    return [tasks[(i * len(tasks)) // n:((i + 1) * len(tasks)) // n] for i in range(n)]


def _twice(d):
    return jnp.concatenate([d, d], axis=0).astype(bf16)


def make(only=None, scopes=False, mc_rel=0.1, b1_ln=4, b_ln=0.8, kv_late=4, ln5=3, ln7=3):
    ln_late = {5: ln5, 7: ln7}

    def kernel(q_hbm, k_hbm, v_hbm, sk_hbm, hk_hbm, dv_hbm, w1_hbm, w2_hbm, w3_hbm, w4_hbm,
               o_hbm,
               qb, kb, vb, hkb, w1, w2, w3, w4, sk_ref, dv_ref, ff, fi, skt, hprev, U, G, Yb,
               xb, ybuf, hs3, xab, xinb, zbuf, obuf, ubuf, tbuf, kst, baseb, accb,
               sems):
        def is_static(j):
            return isinstance(j, int)

        def rows_at(r0, n):
            return pl.ds(r0 if is_static(r0) else pl.multiple_of(r0, n), n)

        def rem(j, n):
            return j % n if is_static(j) else lax.rem(j, n)

        def hk(j):
            return [pltpu.make_async_copy(hk_hbm.at[:, pl.ds(j * TM, TM)], hkb.at[j % NIN], sems.at[j])]

        def kv_in(j):
            rows = pl.ds(j * TM, TM)
            return [pltpu.make_async_copy(k_hbm.at[0, rows, :], kb.at[j % NIN], sems.at[T + j]),
                    pltpu.make_async_copy(v_hbm.at[0, rows, :], vb.at[j % NIN], sems.at[2 * T + j])]

        def tile(j):
            return hk(j) + kv_in(j)

        def qs(j):
            rows = pl.ds(j * TM, TM)
            return [pltpu.make_async_copy(q_hbm.at[0, rows, :], qb.at[rows, :], sems.at[3 * T + j])]

        def whole(i):
            src, dst = [(w1_hbm, w1), (w2_hbm, w2), (sk_hbm, sk_ref), (dv_hbm, dv_ref)][i]
            return [pltpu.make_async_copy(src, dst, sems.at[4 * T + i])]

        def chunks(lo, hi):
            out = []
            for c in range(lo, hi):
                cs = pl.ds(c * FC, FC)
                out += [pltpu.make_async_copy(w3_hbm.at[:, cs], w3.at[:, cs], sems.at[4 * T + 4 + 2 * c]),
                        pltpu.make_async_copy(w4_hbm.at[cs, :], w4.at[cs, :], sems.at[4 * T + 5 + 2 * c])]
            return out

        def out_copy(j):
            rows = rows_at(j * TM, TM)
            return pltpu.make_async_copy(obuf.at[rows, :], o_hbm.at[0, rows, :], sems.at[4 * T + 4 + 2 * NFC + j])

        def last_copy(n):
            rows = pl.ds((T - 1) * TM, TM)
            cs = pl.ds(n * (D // NLAST), D // NLAST)
            return pltpu.make_async_copy(obuf.at[rows, cs], o_hbm.at[0, rows, cs], sems.at[5 * T + 3 + 2 * NFC + n])

        def start_all(cps):
            for cp in cps:
                cp.start()

        def wait_all(cps):
            for cp in cps:
                cp.wait()

        z = jnp.min(lax.broadcasted_iota(jnp.int32, (8, 128), 1))
        never = z > 0
        z16 = pl.multiple_of(z, 16)

        def need(w, dls):
            dls = [d for d in dls if d is not None]
            if not dls:
                return w
            nt = w.shape[1] // 128
            cols = [w[:, n * 128:(n + 1) * 128] for n in range(nt)]
            npass = w.shape[0] // 512
            used = {}
            for i, d in enumerate(dls):
                slot = ((i + 1) * nt * npass - 1) // len(dls)
                used[slot] = used.get(slot, -1) + 1
                n, r0 = slot // npass, (slot % npass) * 512 + 16 * used[slot]
                parts = [cols[n][:r0]] if r0 else []
                parts += [jnp.where(never, d, cols[n][r0:r0 + 16]), cols[n][r0 + 16:]]
                cols[n] = jnp.concatenate(parts, axis=0)
            return jnp.concatenate(cols, axis=1)

        def after(x, srcs):
            if not srcs:
                return x
            head = jnp.where(never, _twice(srcs[max(0, len(srcs) - 33)]()), x[:16, :128])
            if x.shape[1] > 128:
                head = jnp.concatenate([head, x[:16, 128:]], axis=1)
            return jnp.concatenate([head, x[16:]], axis=0)

        def release_k(srcs):
            for i in range(32):
                kb[z + NIN, 16 * (i // 8):16 * (i // 8) + 16, (i % 8) * 128:(i % 8 + 1) * 128] = _twice(srcs[i]())

        def release_u(srcs):
            for i in range(32):
                U[z + NB, 8 * i:8 * i + 8, 0:128] = srcs[i]()

        def release_g(srcs):
            for i in range(32):
                G[z + NB - 1, 8 * i:8 * i + 8, 0:128] = srcs[i]()

        def constants():
            r = lax.broadcasted_iota(jnp.int32, (2 * PB, PB), 0)
            t = lax.broadcasted_iota(jnp.int32, (2 * PB, PB), 1)
            slot = ((r >> 4) << 3) + (r & 7)
            freq = jnp.where(slot < 64, 2 * slot, 2 * slot - 127)
            phase = ((2 * freq + 1) * t + jnp.where((r & 8) != 0, 128, 0)) & 511
            fw = jnp.cos(phase.astype(f32) * (2.0 * math.pi / 512.0))
            ff[...] = fw.astype(bf16)
            fi[...] = (fw.T * (1.0 / PB)).astype(bf16)
            kst[:, 0:16, :] = jnp.zeros((4, 16, 128), f32)
            hs3[1, 0:8, :] = jnp.zeros((8, D), f32)
            hs3[T, TM - 8:TM, :] = jnp.zeros((8, D), f32)

        def job_h(j, prev=()):
            ffv = after(ff[...], prev)
            srcs = []
            LQ = D // 4
            for qd in range(4):
                ls = slice(qd * LQ, (qd + 1) * LQ)
                hh = _dot_nt(ffv, jnp.concatenate([hkb[j % NIN, ls, 0:PB], hkb[j % NIN, ls, PB:2 * PB]], axis=0))
                srcs += _pieces(hh, 4)
                for g in range(PB // 8):
                    re, im = hh[16 * g:16 * g + 8], hh[16 * g + 8:16 * g + 16]
                    blocks = [(re[:, :LQ], im[:, :LQ]), (re[:, LQ:], im[:, LQ:])]
                    for i in range(2):
                        gr, gi = blocks[i]
                        if 2 * j + i > 0:
                            pr, pi_ = blocks[0] if i else (hprev[16 * g:16 * g + 8, ls],
                                                           hprev[16 * g + 8:16 * g + 16, ls])
                            gr, gi = (gr - pi_, gi + pr) if g < 8 else (gr + pi_, gi - pr)
                        G[2 * j + i, 8 * g:8 * g + 8, ls] = gr
                        G[2 * j + i, PB + 8 * g:PB + 8 * g + 8, ls] = gi - gr
                        G[2 * j + i, 2 * PB + 8 * g:2 * PB + 8 * g + 8, ls] = gr + gi
                    if j < T - 1:
                        hprev[16 * g:16 * g + 16, ls] = hh[16 * g:16 * g + 16, LQ:]
            return srcs

        def tasks_kv(j):
            sl = j % NIN

            def task(i, lt, gate=None):
                ls = slice(lt * 128, (lt + 1) * 128)
                rs = slice(i * PB, (i + 1) * PB)
                if gate is not None:
                    kb[z + NIN, pl.ds(z16, 16), ls] = _twice(gate)
                kf = kb[sl, rs, ls].astype(f32)
                pair, par = lt // 2, lt % 2
                kst[pair, pl.ds(2 * (8 + i * PB) + par, PB, stride=2), :] = kf
                ks = kf * skt[0:1, ls]
                for tt in range(1, 4):
                    ks = ks + kst[pair, pl.ds(2 * (8 - tt + i * PB) + par, PB, stride=2), :] * skt[tt:tt + 1, ls]
                if i == 1:
                    kst[pair, pl.ds(par, 8, stride=2), :] = kf[PB - 8:]
                ubuf[j % 2, rs, ls] = (ks * vb[sl, rs, ls].astype(f32)).astype(bf16)
                return ubuf[j % 2, pl.ds(z16 + i * PB, 16), ls]

            return [_Gated(functools.partial(task, i, lt)) for i in range(2) for lt in range(8)]

        def job_u(j, prev=()):
            ubuf[j % 2, pl.ds(z16 + TM, 16), 0:128] = jnp.zeros((16, 128), bf16)
            ffv = after(ff[...], prev)
            srcs = []
            for i in range(2):
                uu = _dot(ffv, ubuf[j % 2, i * PB:(i + 1) * PB, :])
                srcs += _pieces(uu, 4)
                U[2 * j + i] = uu
            return srcs

        def run_mac(j):
            for r0 in range(0, PB, 8):
                for l0 in range(0, D, 256):
                    ls = slice(l0, l0 + 256)
                    gld = lambda c: [G[c, p * PB + r0:p * PB + r0 + 8, ls] for p in range(3)]
                    acc = [None, None]
                    g = gld(2 * j + 1)
                    for b in range(2 * j + 2):
                        ua, ub = U[b, 2 * r0:2 * r0 + 8, ls], U[b, 2 * r0 + 8:2 * r0 + 16, ls]
                        us = ua + ub
                        for i in (1, 0):
                            if 2 * j + i - b >= 0:
                                if i == 0:
                                    g = gld(2 * j - b)
                                term = [g[0] * us, g[1] * ua, g[2] * ub]
                                acc[i] = term if b == 0 else [x + y for x, y in zip(acc[i], term)]
                    for i in range(2):
                        Yb[i, 2 * r0:2 * r0 + 16, ls] = jnp.concatenate(
                            [acc[i][0] - acc[i][2], acc[i][0] + acc[i][1]], axis=0).astype(bf16)

        def job_inv(j, prev=()):
            Yb[z + 2, 0:16, 0:128] = jnp.zeros((16, 128), bf16)
            fiv = after(fi[...], prev)
            srcs = []
            for i in range(2):
                yc = _dot(fiv, Yb[i])
                srcs += _pieces(yc, 2)
                y = yc + ubuf[j % 2, i * PB:(i + 1) * PB, :].astype(f32) * skt[4:5, :]
                ybuf[j * TM + i * PB:j * TM + (i + 1) * PB, :] = y.astype(bf16)
            return srcs

        def tasks_ln(p, res, gated=False, mem=False):
            j = rem(p, T)
            s3, s4 = rem(p, 3), rem(p, 4)
            res['t'] = [None] * 16

            def task(k, gate=None):
                rows = rows_at(j * TM + k * 16, 16)
                if gate is not None:
                    qb[pl.ds(z16 + S, 16), 0:128] = _twice(gate)
                x = qb[rows, :].astype(f32) if is_static(p) else xb[rows, :]
                xa = x + _ln(x) * ybuf[rows, :].astype(f32)
                xin = _ln(xa)
                res['t'][k] = _ln_centered(xin).astype(bf16)
                if mem:
                    tbuf[p % 2, k * 16:(k + 1) * 16, :] = res['t'][k]
                xab[s3, k * 16:(k + 1) * 16, :] = xa + xin
                xinb[s4, k * 16:(k + 1) * 16, :] = xin
                return res['t'][k][:, 0:128]

            wrap = _Gated if gated else (lambda f: f)
            return [wrap(functools.partial(task, k)) for k in range(16)]

        def tasks_ln2(p):
            def task(k, gate=None):
                if gate is not None:
                    xinb[z + 4, k * 16:(k + 1) * 16, 0:128] = jnp.concatenate([gate, gate], axis=0)
                zv = _ln(xinb[rem(p, 4), k * 16:(k + 1) * 16, :]).astype(bf16)
                zbuf[rem(p, 2), k * 16:(k + 1) * 16, :] = zv
                return zv[:, 0:128]

            return [_Gated(functools.partial(task, k)) for k in range(16)]

        def job_w1(p, res, prev=()):
            tt = tbuf[p % 2] if res is None else jnp.concatenate(res['t'], axis=0)
            pre = _dot(after(tt, prev), w1[...])
            h = _gelu(pre)
            me = rem(p, T) + 1
            for g, sh in enumerate(SHIFTS):
                ls = slice(g * (D // 4), (g + 1) * (D // 4))
                hg = h[:, ls]
                if sh > 0:
                    hs3[me, sh:TM, ls] = hg[0:TM - sh]
                    hs3[me + 1, 0:sh, ls] = hg[TM - sh:TM]
                else:
                    hs3[me, 0:TM + sh, ls] = hg[-sh:TM]
                    hs3[me - 1, TM + sh:TM, ls] = hg[0:-sh]
            return _pieces(pre)

        def job_w2(p):
            s4 = rem(p, 4)
            hs = _dot(hs3[rem(p, T) + 1].astype(bf16), w2[...])
            xinb[z + s4 if is_static(s4) else s4] = xinb[s4] + hs
            baseb[rem(p, 2)] = xab[rem(p, 3)] + hs
            return _pieces(hs)

        def m_begin(p):
            return dict(rows=rows_at(rem(p, T) * TM, TM), s2=rem(p, 2), z=zbuf[rem(p, 2)])

        def job_m(st, c, t3=(), t4=(), flow=None):
            pre = _dot(st['z'], need(w3[:, c * FC:(c + 1) * FC], st.pop('dl', [])))
            hh = _gelu(pre).astype(bf16)
            if flow is not None:
                flow(_pieces(pre))
            part = _dot(hh, need(w4[c * FC:(c + 1) * FC, :], _run(t3, _pieces(pre))))
            st['acc'] = (st['acc'] if c else baseb[st['s2']]) + part
            st['dl'] = _run(t4, _pieces(part))

        def m_jobs(st, tasks):
            parts = _split(tasks, 2 * NFC - 1) + [[]]
            for c in range(NFC):
                job_m(st, c, parts[2 * c], parts[2 * c + 1])

        def step_b0(mid):
            _run(tasks_kv(0))
            prev = job_u(0)
            release_u(prev[-32:])
            run_mac(0)
            job_inv(0, prev)
            mid()
            job_h(1)

        def step_b1():
            res = {}
            _run(tasks_kv(1))
            ln = tasks_ln(0, res, gated=True, mem=True)
            _run(ln[:b1_ln])
            prev = job_u(1)
            release_u(prev[-32:])
            _run(ln[b1_ln:], prev)
            run_mac(1)
            job_inv(1, prev)

        def step_b2(mid):
            prev = job_w1(0, None)
            release_k(prev)
            _run(tasks_kv(2))
            _run(tasks_ln(1, {}, gated=True, mem=True), prev[:int(len(prev) * b_ln)])
            job_u(2, prev)
            mid()
            ph = job_h(2)
            release_g(ph[-32:])
            prev = job_w1(1, None, ph)
            release_u(ph[-32:])
            run_mac(2)
            job_inv(2, prev)

        def step_b3():
            res = {}
            prev = job_w2(0)
            release_k(prev)
            _run(tasks_kv(3))
            _run(tasks_ln(2, res, gated=True), prev[:int(len(prev) * b_ln)])
            prev = job_u(3, prev)
            prev = job_h(3, prev)
            prev = job_w1(2, res, prev)
            _run(tasks_ln2(0), prev[:len(prev) * 3 // 4])

        def tasks_q2x(j):
            def task(k):
                rows = pl.ds(j * TM + k * 32, 32)
                xb[rows, :] = qb[rows, :].astype(f32)
                return xb[pl.ds(z16 + j * TM + k * 32, 16), 0:128].astype(bf16)
            return [functools.partial(task, k) for k in range(TM // 32)]

        def step_mc_a(t, mac, h_first=None, fwd=None, q2x=None):
            st = m_begin(t - 4)
            if h_first is not None:
                release_g(job_h(h_first)[-32:])
            prev = job_w2(t - 3)
            release_u(prev[int(len(prev) * mc_rel):])
            run_mac(mac)
            kv = _split(_interleave(tasks_kv(fwd) if fwd else [], tasks_q2x(q2x) if q2x else []), 3)
            job_m(st, 0)
            job_m(st, 1, kv[0], kv[1])
            job_m(st, 2, _interleave(kv[2], tasks_ln2(t - 3)))
            accb[...] = st['acc']
            job_inv(mac)
            if fwd:
                job_u(fwd)
                job_h(fwd)

        def step_mc_b(t, mid=None, mac=None, kvu=None, h=None):
            res = {}
            st = m_begin(t - 4)
            st['acc'] = accb[...]
            s_ln = 0 if mac is None else ln_late[mac]
            s_kv = 4 if mid else (0 if mac is None else kv_late)
            n_ln = 7 if mac is None else 8
            slots = [[] for _ in range(8)]
            for i, part in enumerate(_split(tasks_ln(t - 1, res), n_ln - s_ln)):
                slots[s_ln + i] = part
            if kvu is not None:
                for i, part in enumerate(_split(tasks_kv(kvu), 7 - s_kv)):
                    slots[s_kv + i] = _interleave(slots[s_kv + i], part)
            for c in range(3, NFC):
                if mid and c == 5:
                    mid()
                job_m(st, c, slots[2 * (c - 3)], slots[2 * (c - 3) + 1],
                      flow=(lambda srcs: (release_u(srcs), run_mac(mac))) if c == 3 and mac is not None else None)
            if mac is not None:
                job_inv(mac)
            if kvu is not None:
                job_u(kvu)
            if h is not None:
                job_h(h)
            xb[st['rows'], :] = st['acc']
            job_w1(t - 1, res)

        def body_mpr(t, carry):
            res = {}
            st = m_begin(t - 4)
            job_w2(t - 3)
            m_jobs(st, tasks_ln2(t - 3) + tasks_ln(t - 1, res))
            xb[st['rows'], :] = st['acc']
            obuf[st['rows'], :] = st['acc'].astype(bf16)
            job_w1(t - 1, res)

            @pl.when(t - 4 >= T)
            def _():
                out_copy(t - 4 - T).start()
            return carry

        def body_mr(t, carry):
            st = m_begin(t - 4)
            job_w2(t - 3)
            m_jobs(st, tasks_ln2(t - 3))
            obuf[st['rows'], :] = st['acc'].astype(bf16)
            out_copy(t - 4 - T).start()
            return carry

        def step_last():
            st = m_begin(2 * T - 1)
            m_jobs(st, [])
            for n in range(NLAST):
                cs = slice(n * (D // NLAST), (n + 1) * (D // NLAST))
                obuf[st['rows'], cs] = st['acc'][:, cs].astype(bf16)
                last_copy(n).start()

        scope = jax.named_scope if scopes else (lambda name: contextlib.nullcontext())
        nreg = [0]

        def region(name, fn, *args):
            nreg[0] += 1
            with scope(name):
                pl.when(z <= nreg[0])(lambda: (fn(*args), None)[1])

        def waits(name, cps):
            with scope("w" + name):
                wait_all(cps)

        parts = {
            '4a': lambda: step_mc_a(4, 3),
            '4b': lambda mid: step_mc_b(4, mid, kvu=4, h=4),
            '5a': lambda: step_mc_a(5, 4, fwd=5, q2x=6),
            '5b': lambda: step_mc_b(5, mac=5, kvu=6),
            '6a': lambda: step_mc_a(6, 6, h_first=6, fwd=7, q2x=7),
            '6b': lambda: step_mc_b(6, mac=7),
        }

        start_all(hk(0) + whole(2) + whole(3) + kv_in(0) + hk(1) + kv_in(1) + qs(0) + whole(0) + qs(1)
                  + kv_in(2) + hk(2) + whole(1) + hk(3) + qs(2) + kv_in(3))
        region("const", constants)
        waits("h0", hk(0))
        region("h0", job_h, 0)
        wait_all(whole(2) + whole(3))
        skt[0:4, :] = sk_ref[...].astype(f32)
        skt[4:8, :] = jnp.broadcast_to(dv_ref[...].astype(f32).reshape(1, D), (4, D))
        waits("b0", kv_in(0))
        region("b0", step_b0, lambda: wait_all(hk(1)))
        start_all(chunks(0, 4) + qs(3) + chunks(4, NFC) + tile(4))
        waits("b1", kv_in(1) + qs(0))
        region("b1", step_b1)
        start_all(qs(4) + tile(5))
        waits("b2", whole(0) + qs(1) + kv_in(2))
        region("b2", step_b2, lambda: wait_all(hk(2)))
        start_all(qs(5) + tile(6))
        waits("b3", whole(1) + hk(3) + qs(2) + kv_in(3))
        region("b3", step_b3)
        start_all(qs(6) + tile(7) + qs(7))
        waits("4a", chunks(0, 3))
        region("mc4a", parts['4a'])
        waits("4b", chunks(3, 4) + qs(3) + chunks(4, 5))
        region("mc4b", parts['4b'], lambda: wait_all(chunks(5, NFC) + tile(4)))
        waits("5a", tile(5) + qs(6))
        region("mc5a", parts['5a'])
        waits("5b", qs(4) + tile(6))
        region("mc5b", parts['5b'])
        waits("6a", tile(7) + qs(7))
        region("mc6a", parts['6a'])
        waits("6b", qs(5))
        region("mc6b", parts['6b'])
        with scope("loopMPR"):
            lax.fori_loop(T - 1, 2 * T + 1, body_mpr, 0)
        with scope("loopMR"):
            lax.fori_loop(2 * T + 1, 2 * T + 3, body_mr, 0)
        with scope("last"):
            step_last()
        with scope("waitO"):
            wait_all([out_copy(j) for j in range(T - 1)] + [last_copy(n) for n in range(NLAST)])

    @jax.jit
    def fn(A_q, A_k, A_v, A_shift_k, A_ssm_k, A_ssm_D, B_x, B_w1, B_w2, B_w3, B_w4):
        scratch = [
            pltpu.VMEM((S + 16, D), bf16),
            pltpu.VMEM((NIN + 1, TM, D), bf16),
            pltpu.VMEM((NIN, TM, D), bf16),
            pltpu.VMEM((NIN, D, TM), bf16),
            pltpu.VMEM((D, D), bf16),
            pltpu.VMEM((D, D), bf16),
            pltpu.VMEM((D, F), bf16),
            pltpu.VMEM((F, D), bf16),
            pltpu.VMEM((4, D), bf16),
            pltpu.VMEM((D,), bf16),
            pltpu.VMEM((2 * PB, PB), bf16),
            pltpu.VMEM((PB, 2 * PB), bf16),
            pltpu.VMEM((8, D), f32),
            pltpu.VMEM((2 * PB, D), f32),
            pltpu.VMEM((NB + 1, 2 * PB, D), f32),
            pltpu.VMEM((NB, 3 * PB, D), f32),
            pltpu.VMEM((3, 2 * PB, D), bf16),
            pltpu.VMEM((S, D), f32),
            pltpu.VMEM((S, D), bf16),
            pltpu.VMEM((T + 2, TM, D), f32),
            pltpu.VMEM((3, TM, D), f32),
            pltpu.VMEM((5, TM, D), f32),
            pltpu.VMEM((2, TM, D), bf16),
            pltpu.VMEM((S, D), bf16),
            pltpu.VMEM((2, TM + 16, D), bf16),
            pltpu.VMEM((2, TM, D), bf16),
            pltpu.VMEM((4, 2 * (TM + 16), 128), f32),
            pltpu.VMEM((2, TM, D), f32),
            pltpu.VMEM((TM, D), f32),
            pltpu.SemaphoreType.DMA((5 * T + 3 + 2 * NFC + NLAST,)),
        ]
        return pl.pallas_call(
            kernel,
            in_specs=[pl.BlockSpec(memory_space=pl.ANY)] * 10,
            out_specs=pl.BlockSpec(memory_space=pl.ANY),
            out_shape=jax.ShapeDtypeStruct((1, S, D), bf16),
            scratch_shapes=scratch,
            compiler_params=pltpu.CompilerParams(vmem_limit_bytes=124 * 1024 * 1024),
        )(A_q, A_k, A_v, A_shift_k.T, A_ssm_k, A_ssm_D, B_w1, B_w2, B_w3, B_w4)

    return fn


_impl = make()


@jax.jit
def pallas_interleave_layers__ssm_conv_h3__mixer_s_mlp__prompt_kernel(
        A_q, A_k, A_v, A_shift_k, A_ssm_k, A_ssm_D, B_x, B_w1, B_w2, B_w3, B_w4):
    return _impl(A_q, A_k, A_v, A_shift_k, A_ssm_k, A_ssm_D, B_x, B_w1, B_w2, B_w3, B_w4)
```

```python
import contextlib
import functools
import math

import jax
import jax.numpy as jnp
from jax import lax
import jax.experimental.pallas as pl
import jax.experimental.pallas.tpu as pltpu

S = 2048
D = 1024
F = 3584
TM = 256
T = S // TM
PB = 128
NB = S // PB
FC = 512
NFC = F // FC
EPS = 1e-5
SHIFTS = (1, -1, 2, -2)
NIN = 4
NLAST = 4
f32 = jnp.float32
bf16 = jnp.bfloat16


def _ln(x):
    m = jnp.mean(x, axis=-1, keepdims=True)
    xc = x - m
    v = jnp.mean(xc * xc, axis=-1, keepdims=True)
    return xc * lax.rsqrt(v + EPS)


def _ln_centered(x):
    n = x.shape[-1]
    m = jnp.sum(x, axis=-1, keepdims=True) * (1.0 / n)
    ms = jnp.sum(x * x, axis=-1, keepdims=True) * (1.0 / n)
    v = jnp.maximum(ms - m * m, 0.0)
    return (x - m) * lax.rsqrt(v + EPS)


def _gelu(x):
    c = math.sqrt(2.0 / math.pi)
    inner = x * (c + (c * 0.044715) * (x * x))
    hx = 0.5 * x
    return hx + hx * jnp.tanh(inner)


def _dot(a, b):
    return jnp.dot(a, b, preferred_element_type=f32)


def _dot_nt(a, b):
    return lax.dot_general(a, b, (((1,), (1,)), ((), ())), preferred_element_type=f32)


def _pieces(val, ngroup=1):
    rows, cols = val.shape
    return [functools.partial(lambda r, n: val[r * 8:(r + 1) * 8, n * 128:(n + 1) * 128], r, n)
            for n in range(0, cols // 128, ngroup) for r in range(rows // 8)]


class _Gated:
    def __init__(self, fn):
        self.fn = fn

    def __call__(self, gate=None):
        return self.fn(gate=gate)


def _run(tasks, srcs=None):
    out = []
    for i, task in enumerate(tasks):
        if srcs and isinstance(task, _Gated):
            out.append(task(srcs[(i * len(srcs)) // len(tasks)]()))
        else:
            out.append(task())
    return out


def _interleave(*lists):
    items = [((i + 0.5) / len(l), li, x) for li, l in enumerate(lists) for i, x in enumerate(l)]
    items.sort(key=lambda e: (e[0], e[1]))
    return [e[2] for e in items]


def _split(tasks, n):
    return [tasks[(i * len(tasks)) // n:((i + 1) * len(tasks)) // n] for i in range(n)]


def _reverse_rows(x):
    groups = []
    for g in range(x.shape[0] // 8 - 1, -1, -1):
        v = x[g * 8:(g + 1) * 8]
        r = lax.broadcasted_iota(jnp.int32, v.shape, 0)
        v = jnp.where((r & 1) == 0, pltpu.roll(v, 1, 0), pltpu.roll(v, 3, 0))
        groups.append(jnp.where((r & 2) == 0, v, pltpu.roll(v, 4, 0)))
    return jnp.concatenate(groups, axis=0)


def _twice(d):
    return jnp.concatenate([d, d], axis=0).astype(bf16)


def make(only=None, scopes=False, mc_rel=0.1, b1_ln=4, b_ln=0.75, kv_late=4, ln5=3, ln7=3):
    ln_late = {5: ln5, 7: ln7}

    def kernel(q_hbm, k_hbm, v_hbm, sk_hbm, hk_hbm, dv_hbm, w1_hbm, w2_hbm, w3_hbm, w4_hbm,
               o_hbm,
               qb, kb, vb, hkb, w1, w2, w3, w4, sk_ref, dv_ref, ffh, ffu, fi, skt, hprev, U, G, Yb,
               xb, ybuf, hs3, xab, xinb, zbuf, obuf, ubuf, tbuf, kst, baseb, accb,
               sems):
        def is_static(j):
            return isinstance(j, int)

        def rows_at(r0, n):
            return pl.ds(r0 if is_static(r0) else pl.multiple_of(r0, n), n)

        def rem(j, n):
            return j % n if is_static(j) else lax.rem(j, n)

        def hk(j):
            return [pltpu.make_async_copy(hk_hbm.at[:, pl.ds(j * TM, TM)], hkb.at[j % NIN], sems.at[j])]

        def kv_in(j):
            rows = pl.ds(j * TM, TM)
            return [pltpu.make_async_copy(k_hbm.at[0, rows, :], kb.at[j % NIN], sems.at[T + j]),
                    pltpu.make_async_copy(v_hbm.at[0, rows, :], vb.at[j % NIN], sems.at[2 * T + j])]

        def tile(j):
            return hk(j) + kv_in(j)

        def qs(j):
            rows = pl.ds(j * TM, TM)
            return [pltpu.make_async_copy(q_hbm.at[0, rows, :], qb.at[rows, :], sems.at[3 * T + j])]

        def whole(i):
            src, dst = [(w1_hbm, w1), (w2_hbm, w2), (sk_hbm, sk_ref), (dv_hbm, dv_ref)][i]
            return [pltpu.make_async_copy(src, dst, sems.at[4 * T + i])]

        def chunks(lo, hi):
            out = []
            for c in range(lo, hi):
                cs = pl.ds(c * FC, FC)
                out += [pltpu.make_async_copy(w3_hbm.at[:, cs], w3.at[:, cs], sems.at[4 * T + 4 + 2 * c]),
                        pltpu.make_async_copy(w4_hbm.at[cs, :], w4.at[cs, :], sems.at[4 * T + 5 + 2 * c])]
            return out

        def out_copy(j):
            rows = rows_at(j * TM, TM)
            return pltpu.make_async_copy(obuf.at[rows, :], o_hbm.at[0, rows, :], sems.at[4 * T + 4 + 2 * NFC + j])

        def last_copy(n):
            rows = pl.ds((T - 1) * TM, TM)
            cs = pl.ds(n * (D // NLAST), D // NLAST)
            return pltpu.make_async_copy(obuf.at[rows, cs], o_hbm.at[0, rows, cs], sems.at[5 * T + 3 + 2 * NFC + n])

        def start_all(cps):
            for cp in cps:
                cp.start()

        def wait_all(cps):
            for cp in cps:
                cp.wait()

        z = jnp.min(lax.broadcasted_iota(jnp.int32, (8, 128), 1))
        never = z > 0
        z16 = pl.multiple_of(z, 16)

        def need(w, dls):
            dls = [d for d in dls if d is not None]
            if not dls:
                return w
            nt = w.shape[1] // 128
            cols = [w[:, n * 128:(n + 1) * 128] for n in range(nt)]
            npass = w.shape[0] // 512
            used = {}
            for i, d in enumerate(dls):
                slot = ((i + 1) * nt * npass - 1) // len(dls)
                used[slot] = used.get(slot, -1) + 1
                n, r0 = slot // npass, (slot % npass) * 512 + 16 * used[slot]
                parts = [cols[n][:r0]] if r0 else []
                parts += [jnp.where(never, d, cols[n][r0:r0 + 16]), cols[n][r0 + 16:]]
                cols[n] = jnp.concatenate(parts, axis=0)
            return jnp.concatenate(cols, axis=1)

        def after(x, srcs):
            if not srcs:
                return x
            head = jnp.where(never, _twice(srcs[max(0, len(srcs) - 33)]()), x[:16, :128])
            if x.shape[1] > 128:
                head = jnp.concatenate([head, x[:16, 128:]], axis=1)
            return jnp.concatenate([head, x[16:]], axis=0)

        def release_k(srcs):
            for i in range(32):
                kb[z + NIN, 16 * (i // 8):16 * (i // 8) + 16, (i % 8) * 128:(i % 8 + 1) * 128] = _twice(srcs[i]())

        def release_u(srcs):
            for i in range(32):
                U[z + NB, 8 * i:8 * i + 8, 0:128] = srcs[i]()

        def release_g(srcs):
            for i in range(32):
                G[z + NB - 1, 8 * i:8 * i + 8, 0:128] = srcs[i]()

        def dft_matrix(half):
            r = lax.broadcasted_iota(jnp.int32, (2 * PB, PB), 0)
            t = lax.broadcasted_iota(jnp.int32, (2 * PB, PB), 1)
            slot = ((r >> 4) << 3) + (r & 7)
            freq = jnp.where(slot < 64, 2 * slot, 2 * slot - 127)
            phase = ((2 * freq + 1) * (2 * t + half) + jnp.where((r & 8) != 0, 256, 0)) & 1023
            return jnp.cos(phase.astype(f32) * (2.0 * math.pi / 1024.0))

        def constants_h():
            ffh[...] = dft_matrix(0).astype(bf16)

        def constants_u():
            fw = dft_matrix(1)
            ffu[...] = fw.astype(bf16)
            c = jnp.concatenate([fw[16 * g:16 * g + 8] for g in range(PB // 8)], axis=0)
            ns = jnp.concatenate([fw[16 * g + 8:16 * g + 16] for g in range(PB // 8)], axis=0)
            cms, ncps = (c + ns) * (0.5 / PB), (ns - c) * (0.5 / PB)
            fi[:, 0:PB] = jnp.concatenate([ncps[:64], cms[64:]], axis=0).T[:64].astype(bf16)
            fi[:, PB:2 * PB] = jnp.concatenate([cms[:64], ncps[64:]], axis=0).T[:64].astype(bf16)
            kst[:, 0:16, :] = jnp.zeros((4, 16, 128), f32)
            hs3[1, 0:8, :] = jnp.zeros((8, D), f32)
            hs3[T, TM - 8:TM, :] = jnp.zeros((8, D), f32)

        def job_h(j, prev=()):
            ffv = after(ffh[...], prev)
            srcs = []
            LQ = D // 4
            for qd in range(4):
                ls = slice(qd * LQ, (qd + 1) * LQ)
                hh = _dot_nt(ffv, jnp.concatenate([hkb[j % NIN, ls, 0:PB], hkb[j % NIN, ls, PB:2 * PB]], axis=0))
                srcs += _pieces(hh, 4)
                for g in range(PB // 8):
                    re, im = hh[16 * g:16 * g + 8], hh[16 * g + 8:16 * g + 16]
                    blocks = [(re[:, :LQ], im[:, :LQ]), (re[:, LQ:], im[:, LQ:])]
                    for i in range(2):
                        gr, gi = blocks[i]
                        if 2 * j + i > 0:
                            pr, pi_ = blocks[0] if i else (hprev[16 * g:16 * g + 8, ls],
                                                           hprev[16 * g + 8:16 * g + 16, ls])
                            gr, gi = (gr - pi_, gi + pr) if g < 8 else (gr + pi_, gi - pr)
                        G[2 * j + i, 8 * g:8 * g + 8, ls] = gr
                        G[2 * j + i, PB + 8 * g:PB + 8 * g + 8, ls] = gi - gr
                        G[2 * j + i, 2 * PB + 8 * g:2 * PB + 8 * g + 8, ls] = gr + gi
                    if j < T - 1:
                        hprev[16 * g:16 * g + 16, ls] = hh[16 * g:16 * g + 16, LQ:]
            return srcs

        def tasks_kv(j):
            sl = j % NIN

            def task(i, lt, gate=None):
                ls = slice(lt * 128, (lt + 1) * 128)
                rs = slice(i * PB, (i + 1) * PB)
                if gate is not None:
                    kb[z + NIN, pl.ds(z16, 16), ls] = _twice(gate)
                kf = kb[sl, rs, ls].astype(f32)
                pair, par = lt // 2, lt % 2
                kst[pair, pl.ds(2 * (8 + i * PB) + par, PB, stride=2), :] = kf
                ks = kf * skt[0:1, ls]
                for tt in range(1, 4):
                    ks = ks + kst[pair, pl.ds(2 * (8 - tt + i * PB) + par, PB, stride=2), :] * skt[tt:tt + 1, ls]
                if i == 1:
                    kst[pair, pl.ds(par, 8, stride=2), :] = kf[PB - 8:]
                ubuf[j % 2, rs, ls] = (ks * vb[sl, rs, ls].astype(f32)).astype(bf16)
                return ubuf[j % 2, pl.ds(z16 + i * PB, 16), ls]

            return [_Gated(functools.partial(task, i, lt)) for i in range(2) for lt in range(8)]

        def job_u(j, prev=()):
            ubuf[j % 2, pl.ds(z16 + TM, 16), 0:128] = jnp.zeros((16, 128), bf16)
            ffv = after(ffu[...], prev)
            srcs = []
            for i in range(2):
                uu = _dot(ffv, ubuf[j % 2, i * PB:(i + 1) * PB, :])
                srcs += _pieces(uu, 4)
                U[2 * j + i] = uu
            return srcs

        def run_mac(j):
            for r0 in range(0, PB, 8):
                for l0 in range(0, D, 256):
                    ls = slice(l0, l0 + 256)
                    gld = lambda c: [G[c, p * PB + r0:p * PB + r0 + 8, ls] for p in range(3)]
                    acc = [None, None]
                    g = gld(2 * j + 1)
                    for b in range(2 * j + 2):
                        ua, ub = U[b, 2 * r0:2 * r0 + 8, ls], U[b, 2 * r0 + 8:2 * r0 + 16, ls]
                        us = ua + ub
                        for i in (1, 0):
                            if 2 * j + i - b >= 0:
                                if i == 0:
                                    g = gld(2 * j - b)
                                term = [g[0] * us, g[1] * ua, g[2] * ub]
                                acc[i] = term if b == 0 else [x + y for x, y in zip(acc[i], term)]
                    for i in range(2):
                        k1, k2, k3 = acc[i]
                        dif, tot = k2 + k3, (k1 + k1) + (k2 - k3)
                        ya, yb = (dif, tot) if r0 < 64 else (tot, dif)
                        Yb[i, r0:r0 + 8, ls] = ya.astype(bf16)
                        Yb[i, PB + r0:PB + r0 + 8, ls] = yb.astype(bf16)

        def job_inv(j, prev=()):
            Yb[z + 2, 0:16, 0:128] = jnp.zeros((16, 128), bf16)
            fiv = after(fi[...], prev)
            srcs = []
            for i in range(2):
                for l0 in range(0, D, 256):
                    ls = slice(l0, l0 + 256)
                    ys = _dot(fiv[:, 0:PB], Yb[i, 0:PB, ls])
                    yd = _dot(fiv[:, PB:2 * PB], Yb[i, PB:2 * PB, ls])
                    srcs += _pieces(yd, 4)
                    yc = jnp.concatenate([ys + yd, _reverse_rows(ys - yd)], axis=0)
                    y = yc + ubuf[j % 2, i * PB:(i + 1) * PB, ls].astype(f32) * skt[4:5, ls]
                    ybuf[j * TM + i * PB:j * TM + (i + 1) * PB, ls] = y.astype(bf16)
            return srcs

        def tasks_ln(p, res, gated=False, mem=False):
            j = rem(p, T)
            s3, s4 = rem(p, 3), rem(p, 4)
            res['t'] = [None] * 16

            def task(k, gate=None):
                rows = rows_at(j * TM + k * 16, 16)
                if gate is not None:
                    qb[pl.ds(z16 + S, 16), 0:128] = _twice(gate)
                x = qb[rows, :].astype(f32) if is_static(p) else xb[rows, :]
                xa = x + _ln(x) * ybuf[rows, :].astype(f32)
                xin = _ln(xa)
                res['t'][k] = _ln_centered(xin).astype(bf16)
                if mem:
                    tbuf[p % 2, k * 16:(k + 1) * 16, :] = res['t'][k]
                xab[s3, k * 16:(k + 1) * 16, :] = xa + xin
                xinb[s4, k * 16:(k + 1) * 16, :] = xin
                return res['t'][k][:, 0:128]

            wrap = _Gated if gated else (lambda f: f)
            return [wrap(functools.partial(task, k)) for k in range(16)]

        def tasks_ln2(p):
            def task(k, gate=None):
                if gate is not None:
                    xinb[z + 4, k * 16:(k + 1) * 16, 0:128] = jnp.concatenate([gate, gate], axis=0)
                zv = _ln(xinb[rem(p, 4), k * 16:(k + 1) * 16, :]).astype(bf16)
                zbuf[rem(p, 2), k * 16:(k + 1) * 16, :] = zv
                return zv[:, 0:128]

            return [_Gated(functools.partial(task, k)) for k in range(16)]

        def job_w1(p, res, prev=()):
            tt = tbuf[p % 2] if res is None else jnp.concatenate(res['t'], axis=0)
            pre = _dot(after(tt, prev), w1[...])
            h = _gelu(pre)
            me = rem(p, T) + 1
            for g, sh in enumerate(SHIFTS):
                ls = slice(g * (D // 4), (g + 1) * (D // 4))
                hg = h[:, ls]
                if sh > 0:
                    hs3[me, sh:TM, ls] = hg[0:TM - sh]
                    hs3[me + 1, 0:sh, ls] = hg[TM - sh:TM]
                else:
                    hs3[me, 0:TM + sh, ls] = hg[-sh:TM]
                    hs3[me - 1, TM + sh:TM, ls] = hg[0:-sh]
            return _pieces(pre)

        def job_w2(p):
            s4 = rem(p, 4)
            hs = _dot(hs3[rem(p, T) + 1].astype(bf16), w2[...])
            xinb[z + s4 if is_static(s4) else s4] = xinb[s4] + hs
            baseb[rem(p, 2)] = xab[rem(p, 3)] + hs
            return _pieces(hs)

        def m_begin(p):
            return dict(rows=rows_at(rem(p, T) * TM, TM), s2=rem(p, 2), z=zbuf[rem(p, 2)])

        def job_m(st, c, t3=(), t4=(), flow=None):
            pre = _dot(st['z'], need(w3[:, c * FC:(c + 1) * FC], st.pop('dl', [])))
            hh = _gelu(pre).astype(bf16)
            if flow is not None:
                flow(_pieces(pre))
            part = _dot(hh, need(w4[c * FC:(c + 1) * FC, :], _run(t3, _pieces(pre))))
            st['acc'] = (st['acc'] if c else baseb[st['s2']]) + part
            st['dl'] = _run(t4, _pieces(part))

        def m_jobs(st, tasks):
            parts = _split(tasks, 2 * NFC - 1) + [[]]
            for c in range(NFC):
                job_m(st, c, parts[2 * c], parts[2 * c + 1])

        def step_b0(mid):
            _run(tasks_kv(0))
            prev = job_u(0)
            release_u(prev[-32:])
            run_mac(0)
            job_inv(0, prev)
            mid()
            job_h(1)

        def step_b1():
            res = {}
            _run(tasks_kv(1))
            ln = tasks_ln(0, res, gated=True, mem=True)
            _run(ln[:b1_ln])
            prev = job_u(1)
            release_u(prev[-32:])
            _run(ln[b1_ln:], prev)
            run_mac(1)
            job_inv(1, prev)

        def step_b2(mid):
            prev = job_w1(0, None)
            release_k(prev)
            _run(tasks_kv(2))
            _run(tasks_ln(1, {}, gated=True, mem=True), prev[:int(len(prev) * b_ln)])
            job_u(2, prev)
            mid()
            ph = job_h(2)
            release_g(ph[-32:])
            prev = job_w1(1, None, ph)
            release_u(ph[-32:])
            run_mac(2)
            job_inv(2, prev)

        def step_b3():
            res = {}
            prev = job_w2(0)
            release_k(prev)
            _run(tasks_kv(3))
            _run(tasks_ln(2, res, gated=True), prev[:int(len(prev) * b_ln)])
            prev = job_u(3, prev)
            prev = job_h(3, prev)
            prev = job_w1(2, res, prev)
            _run(tasks_ln2(0), prev[:len(prev) * 3 // 4])

        def tasks_q2x(j):
            def task(k):
                rows = pl.ds(j * TM + k * 32, 32)
                xb[rows, :] = qb[rows, :].astype(f32)
                return xb[pl.ds(z16 + j * TM + k * 32, 16), 0:128].astype(bf16)
            return [functools.partial(task, k) for k in range(TM // 32)]

        def step_mc_a(t, mac, h_first=None, fwd=None, q2x=None):
            st = m_begin(t - 4)
            if h_first is not None:
                release_g(job_h(h_first)[-32:])
            prev = job_w2(t - 3)
            release_u(prev[int(len(prev) * mc_rel):])
            run_mac(mac)
            kv = _split(_interleave(tasks_kv(fwd) if fwd else [], tasks_q2x(q2x) if q2x else []), 3)
            job_m(st, 0)
            job_m(st, 1, kv[0], kv[1])
            job_m(st, 2, _interleave(kv[2], tasks_ln2(t - 3)))
            accb[...] = st['acc']
            job_inv(mac)
            if fwd:
                job_u(fwd)
                job_h(fwd)

        def step_mc_b(t, mid=None, mac=None, kvu=None, h=None):
            res = {}
            st = m_begin(t - 4)
            st['acc'] = accb[...]
            s_ln = 0 if mac is None else ln_late[mac]
            s_kv = 4 if mid else (0 if mac is None else kv_late)
            n_ln = 7 if mac is None else 8
            slots = [[] for _ in range(8)]
            for i, part in enumerate(_split(tasks_ln(t - 1, res), n_ln - s_ln)):
                slots[s_ln + i] = part
            if kvu is not None:
                for i, part in enumerate(_split(tasks_kv(kvu), 7 - s_kv)):
                    slots[s_kv + i] = _interleave(slots[s_kv + i], part)
            for c in range(3, NFC):
                if mid and c == 5:
                    mid()
                job_m(st, c, slots[2 * (c - 3)], slots[2 * (c - 3) + 1],
                      flow=(lambda srcs: (release_u(srcs), run_mac(mac))) if c == 3 and mac is not None else None)
            if mac is not None:
                job_inv(mac)
            if kvu is not None:
                job_u(kvu)
            if h is not None:
                job_h(h)
            xb[st['rows'], :] = st['acc']
            job_w1(t - 1, res)

        def body_mpr(t, carry):
            res = {}
            st = m_begin(t - 4)
            job_w2(t - 3)
            m_jobs(st, tasks_ln2(t - 3) + tasks_ln(t - 1, res))
            xb[st['rows'], :] = st['acc']
            obuf[st['rows'], :] = st['acc'].astype(bf16)
            job_w1(t - 1, res)

            @pl.when(t - 4 >= T)
            def _():
                out_copy(t - 4 - T).start()
            return carry

        def body_mr(t, carry):
            st = m_begin(t - 4)
            job_w2(t - 3)
            m_jobs(st, tasks_ln2(t - 3))
            obuf[st['rows'], :] = st['acc'].astype(bf16)
            out_copy(t - 4 - T).start()
            return carry

        def step_last():
            st = m_begin(2 * T - 1)
            m_jobs(st, [])
            for n in range(NLAST):
                cs = slice(n * (D // NLAST), (n + 1) * (D // NLAST))
                obuf[st['rows'], cs] = st['acc'][:, cs].astype(bf16)
                last_copy(n).start()

        scope = jax.named_scope if scopes else (lambda name: contextlib.nullcontext())
        nreg = [0]

        def region(name, fn, *args):
            nreg[0] += 1
            with scope(name):
                pl.when(z <= nreg[0])(lambda: (fn(*args), None)[1])

        def waits(name, cps):
            with scope("w" + name):
                wait_all(cps)

        parts = {
            '4a': lambda: step_mc_a(4, 3),
            '4b': lambda mid: step_mc_b(4, mid, kvu=4, h=4),
            '5a': lambda: step_mc_a(5, 4, fwd=5, q2x=6),
            '5b': lambda: step_mc_b(5, mac=5, kvu=6),
            '6a': lambda: step_mc_a(6, 6, h_first=6, fwd=7, q2x=7),
            '6b': lambda: step_mc_b(6, mac=7),
        }

        start_all(hk(0) + whole(2) + whole(3) + kv_in(0) + hk(1) + kv_in(1) + qs(0) + whole(0) + qs(1)
                  + kv_in(2) + hk(2) + whole(1) + hk(3) + qs(2) + kv_in(3))
        region("const", constants_h)
        waits("h0", hk(0))
        region("h0", lambda: (job_h(0), constants_u()))
        wait_all(whole(2) + whole(3))
        skt[0:4, :] = sk_ref[...].astype(f32)
        skt[4:8, :] = jnp.broadcast_to(dv_ref[...].astype(f32).reshape(1, D), (4, D))
        waits("b0", kv_in(0))
        region("b0", step_b0, lambda: wait_all(hk(1)))
        start_all(chunks(0, 4) + qs(3) + chunks(4, NFC) + tile(4))
        waits("b1", kv_in(1) + qs(0))
        region("b1", step_b1)
        start_all(qs(4) + tile(5))
        waits("b2", whole(0) + qs(1) + kv_in(2))
        region("b2", step_b2, lambda: wait_all(hk(2)))
        start_all(qs(5) + tile(6))
        waits("b3", whole(1) + hk(3) + qs(2) + kv_in(3))
        region("b3", step_b3)
        start_all(qs(6) + tile(7) + qs(7))
        waits("4a", chunks(0, 3))
        region("mc4a", parts['4a'])
        waits("4b", chunks(3, 4) + qs(3) + chunks(4, 5))
        region("mc4b", parts['4b'], lambda: wait_all(chunks(5, NFC) + tile(4)))
        waits("5a", tile(5) + qs(6))
        region("mc5a", parts['5a'])
        waits("5b", qs(4) + tile(6))
        region("mc5b", parts['5b'])
        waits("6a", tile(7) + qs(7))
        region("mc6a", parts['6a'])
        waits("6b", qs(5))
        region("mc6b", parts['6b'])
        with scope("loopMPR"):
            lax.fori_loop(T - 1, 2 * T + 1, body_mpr, 0)
        with scope("loopMR"):
            lax.fori_loop(2 * T + 1, 2 * T + 3, body_mr, 0)
        with scope("last"):
            step_last()
        with scope("waitO"):
            wait_all([out_copy(j) for j in range(T - 1)] + [last_copy(n) for n in range(NLAST)])

    @jax.jit
    def fn(A_q, A_k, A_v, A_shift_k, A_ssm_k, A_ssm_D, B_x, B_w1, B_w2, B_w3, B_w4):
        scratch = [
            pltpu.VMEM((S + 16, D), bf16),
            pltpu.VMEM((NIN + 1, TM, D), bf16),
            pltpu.VMEM((NIN, TM, D), bf16),
            pltpu.VMEM((NIN, D, TM), bf16),
            pltpu.VMEM((D, D), bf16),
            pltpu.VMEM((D, D), bf16),
            pltpu.VMEM((D, F), bf16),
            pltpu.VMEM((F, D), bf16),
            pltpu.VMEM((4, D), bf16),
            pltpu.VMEM((D,), bf16),
            pltpu.VMEM((2 * PB, PB), bf16),
            pltpu.VMEM((2 * PB, PB), bf16),
            pltpu.VMEM((PB // 2, 2 * PB), bf16),
            pltpu.VMEM((8, D), f32),
            pltpu.VMEM((2 * PB, D), f32),
            pltpu.VMEM((NB + 1, 2 * PB, D), f32),
            pltpu.VMEM((NB, 3 * PB, D), f32),
            pltpu.VMEM((3, 2 * PB, D), bf16),
            pltpu.VMEM((S, D), f32),
            pltpu.VMEM((S, D), bf16),
            pltpu.VMEM((T + 2, TM, D), f32),
            pltpu.VMEM((3, TM, D), f32),
            pltpu.VMEM((5, TM, D), f32),
            pltpu.VMEM((2, TM, D), bf16),
            pltpu.VMEM((S, D), bf16),
            pltpu.VMEM((2, TM + 16, D), bf16),
            pltpu.VMEM((2, TM, D), bf16),
            pltpu.VMEM((4, 2 * (TM + 16), 128), f32),
            pltpu.VMEM((2, TM, D), f32),
            pltpu.VMEM((TM, D), f32),
            pltpu.SemaphoreType.DMA((5 * T + 3 + 2 * NFC + NLAST,)),
        ]
        return pl.pallas_call(
            kernel,
            in_specs=[pl.BlockSpec(memory_space=pl.ANY)] * 10,
            out_specs=pl.BlockSpec(memory_space=pl.ANY),
            out_shape=jax.ShapeDtypeStruct((1, S, D), bf16),
            scratch_shapes=scratch,
            compiler_params=pltpu.CompilerParams(vmem_limit_bytes=124 * 1024 * 1024),
        )(A_q, A_k, A_v, A_shift_k.T, A_ssm_k, A_ssm_D, B_w1, B_w2, B_w3, B_w4)

    return fn


_impl = make()


@jax.jit
def pallas_interleave_layers__ssm_conv_h3__mixer_s_mlp__prompt_kernel(
        A_q, A_k, A_v, A_shift_k, A_ssm_k, A_ssm_D, B_x, B_w1, B_w2, B_w3, B_w4):
    return _impl(A_q, A_k, A_v, A_shift_k, A_ssm_k, A_ssm_D, B_x, B_w1, B_w2, B_w3, B_w4)
```
